```python
import jax
import jax.numpy as jnp

def _softmax(x, axis=-1):
    return jax.nn.softmax(x, axis=axis)

def _gelu(x):
    return jax.nn.gelu(x, approximate=True)

def _silu(x):
    return jax.nn.silu(x)

def _sigmoid(x):
    return jax.nn.sigmoid(x)

def _layernorm(x, axis=-1, eps=1e-05):
    m = jnp.mean(x, axis=axis, keepdims=True)
    v = jnp.var(x, axis=axis, keepdims=True)
    return (x - m) / jnp.sqrt(v + eps)

def _scatter_add(tgt, idx, src, axis=0):
    return tgt.at[idx].add(src)

def _segment_sum(src, seg, n):
    return jax.ops.segment_sum(src, seg, n)

class _Rng:

    def __init__(self, key):
        self._k = key

    def _next(self):
        self._k, sub = jax.random.split(self._k)
        return sub

    def normal(self, shape):
        return jax.random.normal(self._next(), shape, dtype=jnp.bfloat16)

    def randint(self, lo, hi, shape):
        return jax.random.randint(self._next(), shape, lo, hi, dtype=jnp.int32)

    def uniform(self, shape, lo=0.0, hi=1.0):
        return jax.random.uniform(self._next(), shape, jnp.bfloat16, lo, hi)

    def permutation(self, n):
        return jax.random.permutation(self._next(), n)
kernel_name = 'interleave_layers__memory_aug_recurrent_mem_tr__mixer_s_mlp__prompt'

def setup_inputs():
    _rng = _Rng(jax.random.key(int.from_bytes(__import__("os").urandom(4), "little")))
    _w = lambda a: (lambda t: t.astype(jnp.bfloat16) if jnp.issubdtype(t.dtype, jnp.floating) else t)(jnp.asarray(a))

    def _A_setup():
        B, S, Dm = (1, 2048, 640)
        H, Dh = (32, 192)
        M, seg = (8, 32)
        seg = min(seg, S)
        S = S // seg * seg
        return {'x': _w((lambda *s: _rng.normal(s) * 0.05)(B, S, Dm)), 'mem0': _w((lambda *s: _rng.normal(s) * 0.05)(B, M, Dm)), 'Wq': _w((lambda *s: _rng.normal(s) * 0.05)(Dm, H, Dh) * Dm ** (-0.5)), 'Wk': _w((lambda *s: _rng.normal(s) * 0.05)(Dm, H, Dh) * Dm ** (-0.5)), 'Wv': _w((lambda *s: _rng.normal(s) * 0.05)(Dm, H, Dh) * Dm ** (-0.5)), 'Wo': _w((lambda *s: _rng.normal(s) * 0.05)(H, Dh, Dm) * (H * Dh) ** (-0.5)), 'seg_len': seg}
    _A_in = _A_setup()

    def _B_setup():
        B, S, D, F = (1, 2048, 640, 1536)
        return {'x': _w((lambda *s: _rng.normal(s) * 0.05)(B, S, D)), 'w1': _w((lambda *s: _rng.normal(s) * 0.05)(D, D) * D ** (-0.5)), 'w2': _w((lambda *s: _rng.normal(s) * 0.05)(D, D) * D ** (-0.5)), 'w3': _w((lambda *s: _rng.normal(s) * 0.05)(D, F) * D ** (-0.5)), 'w4': _w((lambda *s: _rng.normal(s) * 0.05)(F, D) * F ** (-0.5))}
    _B_in = _B_setup()
    return {'A_x': _A_in['x'], 'A_mem0': _A_in['mem0'], 'A_Wq': _A_in['Wq'], 'A_Wk': _A_in['Wk'], 'A_Wv': _A_in['Wv'], 'A_Wo': _A_in['Wo'], 'A_seg_len': _A_in['seg_len'], 'B_x': _B_in['x'], 'B_w1': _B_in['w1'], 'B_w2': _B_in['w2'], 'B_w3': _B_in['w3'], 'B_w4': _B_in['w4']}

def reference(A_x, A_mem0, A_Wq, A_Wk, A_Wv, A_Wo, A_seg_len, B_x, B_w1, B_w2, B_w3, B_w4):

    def _A_ref(x, mem0, Wq, Wk, Wv, Wo, seg_len):
        B, S, Dm = x.shape
        H, Dh = (Wq.shape[1], Wq.shape[2])
        M = mem0.shape[1]
        scale = Dh ** (-0.5)
        n_seg = S // seg_len
        L = M + seg_len
        idx = jnp.arange(L)
        mask = (idx[:, None] < M) | (idx[:, None] >= idx[None, :])
        mem = mem0
        outs = []
        for s in range(n_seg):
            xs = x[:, s * seg_len:(s + 1) * seg_len, :].copy()
            h = jnp.concatenate([mem, xs], axis=1)
            q = jnp.einsum('btd,dhe->bhte', h, Wq)
            k = jnp.einsum('btd,dhe->bhte', h, Wk)
            v = jnp.einsum('btd,dhe->bhte', h, Wv)
            scores = jnp.einsum('bhqe,bhke->bhqk', q, k) * scale
            scores = jnp.where(mask[None, None], scores, -1000000000.0)
            p = _softmax(scores, axis=-1)
            o = jnp.einsum('bhqk,bhke->bhqe', p, v)
            o = jnp.einsum('bhte,hed->btd', o, Wo)
            mem = o[:, :M, :].copy()
            outs.append(o[:, M:, :])
        return jnp.concatenate(outs, axis=1)

    def _B_ref(x, w1, w2, w3, w4):
        B, S, D = x.shape
        h = _gelu(_layernorm(x, axis=-1) @ w1)
        c = D // 4
        g0 = jnp.pad(h[:, :, 0 * c:1 * c], ((0, 0), (1, 0), (0, 0)))[:, :S, :]
        g1 = jnp.pad(h[:, :, 1 * c:2 * c], ((0, 0), (0, 1), (0, 0)))[:, 1:, :]
        g2 = jnp.pad(h[:, :, 2 * c:3 * c], ((0, 0), (2, 0), (0, 0)))[:, :S, :]
        g3 = jnp.pad(h[:, :, 3 * c:], ((0, 0), (0, 2), (0, 0)))[:, 2:, :]
        hs = jnp.concatenate([g0, g1, g2, g3], axis=-1) @ w2
        x1 = x + hs
        h2 = _gelu(_layernorm(x1, axis=-1) @ w3) @ w4
        return x1 + h2
    x = A_x
    x = x + _A_ref(_layernorm(x, axis=-1), A_mem0, A_Wq, A_Wk, A_Wv, A_Wo, A_seg_len)
    x = x + _B_ref(_layernorm(x, axis=-1), B_w1, B_w2, B_w3, B_w4)
    x = x + _A_ref(_layernorm(x, axis=-1), A_mem0, A_Wq, A_Wk, A_Wv, A_Wo, A_seg_len)
    x = x + _B_ref(_layernorm(x, axis=-1), B_w1, B_w2, B_w3, B_w4)
    return x
```

```python
import functools

import jax
import jax.numpy as jnp
import numpy as np
import jax.experimental.pallas as pl
import jax.experimental.pallas.tpu as pltpu

F32 = jnp.float32
BF16 = jnp.bfloat16
_NEG = -1000000000.0


def _ln(x, eps=1e-05):
    m = jnp.mean(x, axis=-1, keepdims=True)
    d = x - m
    v = jnp.mean(d * d, axis=-1, keepdims=True)
    return d * jax.lax.rsqrt(v + eps)


def _gelu(x):
    c = float(np.sqrt(2.0 / np.pi))
    return 0.5 * x * (1.0 + jnp.tanh(c * (x + 0.044715 * (x * x * x))))


def _dot(a, b):
    return jnp.dot(a, b, preferred_element_type=F32)


def _dot_nt(a, b):
    return jax.lax.dot_general(a, b, (((1,), (1,)), ((), ())), preferred_element_type=F32)


def _make_kernel(S, D, H, Dh, M, SEG, F):
    L = M + SEG
    NSEG = S // SEG
    PW = 2 * Dh
    NP = H // 2
    scale = Dh ** (-0.5)
    RT = 256
    NT = S // RT
    HALO = 8
    c = D // 4

    def kernel(x_ref, mem0_ref, wq_ref, wk_ref, wv_ref, wo_ref,
               w1_ref, w2_ref, w3_ref, w4_ref, out_ref,
               xs_ref, ln_ref, h_ref):
        def init_tile(t, _):
            r = pl.ds(pl.multiple_of(t * RT, RT), RT)
            x = x_ref[r, :].astype(F32)
            xs_ref[r, :] = x
            ln_ref[r, :] = _ln(x)
            return 0
        jax.lax.fori_loop(0, NT, init_tile, 0)
        h_ref[pl.ds(0, HALO), :] = jnp.zeros((HALO, D), F32)
        h_ref[pl.ds(HALO + S, HALO), :] = jnp.zeros((HALO, D), F32)

        def a_step(s, mem):
            r = pl.ds(pl.multiple_of(s * SEG, SEG), SEG)
            hrows = jnp.concatenate([mem, ln_ref[r, :]], axis=0)
            hrows = hrows.astype(BF16).astype(F32)
            lo_pw = jax.lax.broadcasted_iota(jnp.int32, (L, PW), 1) < Dh
            row = jax.lax.broadcasted_iota(jnp.int32, (L, 2 * L), 0)
            col = jax.lax.broadcasted_iota(jnp.int32, (L, 2 * L), 1)
            lo2 = col < L
            colh = jnp.where(lo2, col, col - L)
            mask = (row < M) | (row >= colh)
            acc = jnp.zeros((L, D), F32)
            for j in range(NP):
                cs = slice(j * PW, (j + 1) * PW)
                q = _dot(hrows, wq_ref[:, cs])
                k = _dot(hrows, wk_ref[:, cs])
                v = _dot(hrows, wv_ref[:, cs])
                kst = jnp.concatenate(
                    [jnp.where(lo_pw, k, 0.0), jnp.where(lo_pw, 0.0, k)], axis=0).astype(BF16)
                vst = jnp.concatenate(
                    [jnp.where(lo_pw, v, 0.0), jnp.where(lo_pw, 0.0, v)], axis=0).astype(BF16)
                sc = _dot_nt(q, kst) * scale
                sc = jnp.where(mask, sc, _NEG)
                m_lo = jnp.max(jnp.where(lo2, sc, -jnp.inf), axis=1, keepdims=True)
                m_hi = jnp.max(jnp.where(lo2, -jnp.inf, sc), axis=1, keepdims=True)
                e = jnp.exp(sc - jnp.where(lo2, m_lo, m_hi))
                s_lo = jnp.sum(jnp.where(lo2, e, 0.0), axis=1, keepdims=True)
                s_hi = jnp.sum(jnp.where(lo2, 0.0, e), axis=1, keepdims=True)
                p = e / jnp.where(lo2, s_lo, s_hi)
                o = _dot(p, vst)
                acc = acc + _dot(o, wo_ref[cs, :])
            xs_ref[r, :] = xs_ref[r, :] + acc[M:, :]
            return acc[:M, :]

        def b_pass1(t, _):
            r0 = pl.multiple_of(t * RT, RT)
            xl = _ln(xs_ref[pl.ds(r0, RT), :])
            ln_ref[pl.ds(r0, RT), :] = xl
            h = _gelu(_dot(_ln(xl).astype(BF16), w1_ref[...]))
            h_ref[pl.ds(r0 + HALO, RT), :] = h
            return 0

        def b_pass2(t, last):
            r0 = pl.multiple_of(t * RT, RT)
            pieces = []
            shifts = (-1, 1, -2, 2)
            for lt in range(D // 128):
                c0 = lt * 128
                win = h_ref[pl.ds(r0, RT + 2 * HALO), pl.ds(c0, 128)]
                g_lo, g_hi = c0 // c, min((c0 + 127) // c, 3)
                a = win[HALO + shifts[g_lo]: HALO + shifts[g_lo] + RT]
                if g_hi != g_lo:
                    b = win[HALO + shifts[g_hi]: HALO + shifts[g_hi] + RT]
                    lane = jax.lax.broadcasted_iota(jnp.int32, (RT, 128), 1) + c0
                    a = jnp.where(lane < g_hi * c, a, b)
                pieces.append(a)
            hs_in = jnp.concatenate(pieces, axis=1).astype(BF16)
            x1 = ln_ref[pl.ds(r0, RT), :] + _dot(hs_in, w2_ref[...])
            g = _gelu(_dot(_ln(x1).astype(BF16), w3_ref[...]))
            h2 = _dot(g.astype(BF16), w4_ref[...])
            xn = xs_ref[pl.ds(r0, RT), :] + (x1 + h2)
            if last:
                out_ref[pl.ds(r0, RT), :] = xn.astype(out_ref.dtype)
            else:
                xs_ref[pl.ds(r0, RT), :] = xn
            return 0

        def ln_pass(t, _):
            r = pl.ds(pl.multiple_of(t * RT, RT), RT)
            ln_ref[r, :] = _ln(xs_ref[r, :])
            return 0

        for layer in range(2):
            last = layer == 1
            jax.lax.fori_loop(0, NSEG, a_step, mem0_ref[...].astype(F32))
            jax.lax.fori_loop(0, NT, b_pass1, 0)
            jax.lax.fori_loop(0, NT, functools.partial(_b2_body, b_pass2, last), 0)
            if not last:
                jax.lax.fori_loop(0, NT, ln_pass, 0)

    return kernel


def _b2_body(fn, last, t, carry):
    return fn(t, last)


@functools.partial(jax.jit, static_argnames=("A_seg_len",))
def pallas_interleave_layers__memory_aug_recurrent_mem_tr__mixer_s_mlp__prompt_kernel(
    A_x: jax.Array,
    A_mem0: jax.Array,
    A_Wq: jax.Array,
    A_Wk: jax.Array,
    A_Wv: jax.Array,
    A_Wo: jax.Array,
    A_seg_len,
    B_x: jax.Array,
    B_w1: jax.Array,
    B_w2: jax.Array,
    B_w3: jax.Array,
    B_w4: jax.Array,
):
    del B_x
    B, S, D = A_x.shape
    assert B == 1
    H, Dh = A_Wq.shape[1], A_Wq.shape[2]
    M = A_mem0.shape[1]
    SEG = int(A_seg_len)
    F = B_w3.shape[1]
    kernel = _make_kernel(S, D, H, Dh, M, SEG, F)
    out = pl.pallas_call(
        kernel,
        out_shape=jax.ShapeDtypeStruct((S, D), A_x.dtype),
        scratch_shapes=[
            pltpu.VMEM((S, D), F32),
            pltpu.VMEM((S, D), F32),
            pltpu.VMEM((S + 16, D), F32),
        ],
        compiler_params=pltpu.CompilerParams(vmem_limit_bytes=110 * 1024 * 1024),
    )(
        A_x.reshape(S, D), A_mem0.reshape(M, D),
        A_Wq.reshape(D, H * Dh), A_Wk.reshape(D, H * Dh), A_Wv.reshape(D, H * Dh),
        A_Wo.reshape(H * Dh, D), B_w1, B_w2, B_w3, B_w4,
    )
    return out.reshape(B, S, D)
```

```python
import functools

import jax
import jax.numpy as jnp
import numpy as np
import jax.experimental.pallas as pl
import jax.experimental.pallas.tpu as pltpu

F32 = jnp.float32
BF16 = jnp.bfloat16
I32 = jnp.int32
_NEG = -1000000000.0


def _ln(x, eps=1e-05):
    m = jnp.mean(x, axis=-1, keepdims=True)
    d = x - m
    v = jnp.mean(d * d, axis=-1, keepdims=True)
    return d * jax.lax.rsqrt(v + eps)


def _gelu(x):
    c = float(np.sqrt(2.0 / np.pi))
    return 0.5 * x * (1.0 + jnp.tanh(c * (x + 0.044715 * (x * x * x))))


def _dot(a, b):
    return jnp.dot(a, b, preferred_element_type=F32)


def _dot_nt(a, b):
    return jax.lax.dot_general(a, b, (((1,), (1,)), ((), ())), preferred_element_type=F32)


def _make_kernel(S, D, H, Dh, M, SEG, F, G=8, WO_LAG=3):
    L = M + SEG
    NSEG = S // SEG
    NP = H // 2
    PP = NP // G
    scale = Dh ** (-0.5)
    RT = 256
    NT = S // RT
    HALO = 8
    c = D // 4
    GR = PP * 2 * Dh
    assert Dh == 192 and D % 128 == 0

    def kernel(mem0_ref, x_hbm, wq_hbm, wk_hbm, wv_hbm, wo_hbm,
               w1_hbm, w2_hbm, w3_hbm, w4_hbm, out_ref,
               x_v, stage, wq_s, wk_s, wv_s, wo_ref, w1_ref, w2_ref, w3_ref, w4_ref,
               xs_ref, ln_ref, h_ref, sem_x, sem_st, sem_w):
        cp_x = pltpu.make_async_copy(x_hbm, x_v, sem_x.at[0])
        cp_x.start()
        st_cps = []
        for g in range(G):
            rows = pl.ds(g * GR, GR)
            for mi, w_hbm in enumerate((wq_hbm, wk_hbm, wv_hbm)):
                cp = pltpu.make_async_copy(
                    w_hbm.at[rows], stage.at[mi, rows], sem_st.at[3 * g + mi])
                cp.start()
                st_cps.append(cp)
        w_cps = []
        for wi, (src, dst) in enumerate(((wo_hbm, wo_ref), (w1_hbm, w1_ref), (w2_hbm, w2_ref),
                                         (w3_hbm, w3_ref), (w4_hbm, w4_ref))):
            cp = pltpu.make_async_copy(src, dst, sem_w.at[wi])
            cp.start()
            w_cps.append(cp)

        cp_x.wait()

        def init_tile(t, _):
            r = pl.ds(pl.multiple_of(t * RT, RT), RT)
            x = x_v[r, :].astype(F32)
            xs_ref[r, :] = x
            ln_ref[r, :] = _ln(x)
            return 0
        jax.lax.fori_loop(0, NT, init_tile, 0)
        h_ref[pl.ds(0, HALO), :] = jnp.zeros((HALO, D), F32)
        h_ref[pl.ds(HALO + S, HALO), :] = jnp.zeros((HALO, D), F32)

        for g in range(G):
            for mi, dst in enumerate((wq_s, wk_s, wv_s)):
                st_cps[3 * g + mi].wait()

                def relayout(u, _, mi=mi, g=g, dst=dst):
                    j = g * PP + u
                    r0 = pl.multiple_of(j * 2 * Dh, 128)
                    a = stage[mi, pl.ds(r0, 128), :]
                    b = stage[mi, pl.ds(r0 + Dh, 128), :]
                    t = jnp.concatenate([stage[mi, pl.ds(r0 + 128, 64), :],
                                         stage[mi, pl.ds(r0 + Dh + 128, 64), :]], axis=0)
                    for i, v in enumerate((a, b, t)):
                        dst[3 * j + i] = pltpu.bitcast(v.T, I32)
                    return 0
                jax.lax.fori_loop(0, PP, relayout, 0)
        w_cps[0].wait()

        def a_step(s, mem):
            r = pl.ds(pl.multiple_of(s * SEG, SEG), SEG)
            hrows = jnp.concatenate([mem, ln_ref[r, :]], axis=0)
            lo64 = jax.lax.broadcasted_iota(I32, (L, 128), 1) < 64
            zero = jnp.zeros((L, 128), F32)
            rowb = jax.lax.broadcasted_iota(I32, (PP * L, 2 * L), 0) % L
            colb = jax.lax.broadcasted_iota(I32, (PP * L, 2 * L), 1)
            lob = colb < L
            maskb = (rowb < M) | (rowb >= jnp.where(lob, colb, colb - L))

            def proj(w_s, g):
                w = jnp.concatenate(
                    [pltpu.bitcast(w_s[3 * PP * g + t], BF16) for t in range(3 * PP)], axis=1)
                return _dot(hrows, w)

            def stack(x, j):
                t0 = x[:, 384 * j:384 * j + 128]
                t1 = x[:, 384 * j + 128:384 * j + 256]
                t2 = x[:, 384 * j + 256:384 * j + 384]
                top = jnp.concatenate([t0, zero, jnp.where(lo64, t2, 0.0)], axis=1)
                bot = jnp.concatenate([zero, t1, jnp.where(lo64, 0.0, t2)], axis=1)
                return jnp.concatenate([top, bot], axis=0).astype(BF16)

            def scores(q, k):
                return jnp.concatenate(
                    [_dot_nt(q[:, 384 * j:384 * (j + 1)], stack(k, j)) for j in range(PP)],
                    axis=0) * scale

            def softmax(sc):
                sc = jnp.where(maskb, sc, _NEG)
                m_lo = jnp.max(jnp.where(lob, sc, -jnp.inf), axis=1, keepdims=True)
                m_hi = jnp.max(jnp.where(lob, -jnp.inf, sc), axis=1, keepdims=True)
                e = jnp.exp(sc - jnp.where(lob, m_lo, m_hi))
                s_lo = jnp.sum(jnp.where(lob, e, 0.0), axis=1, keepdims=True)
                s_hi = jnp.sum(jnp.where(lob, 0.0, e), axis=1, keepdims=True)
                return e / jnp.where(lob, s_lo, s_hi)

            def pv(p, v):
                return jnp.concatenate(
                    [_dot(p[j * L:(j + 1) * L], stack(v, j)) for j in range(PP)], axis=1)

            def out_proj(g, o):
                rows = []
                for j in range(PP):
                    r0 = (g * PP + j) * 2 * Dh
                    rows += [wo_ref[r0:r0 + 128, :], wo_ref[r0 + Dh:r0 + Dh + 128, :],
                             wo_ref[r0 + 128:r0 + Dh, :], wo_ref[r0 + Dh + 128:r0 + 2 * Dh, :]]
                return _dot(o, jnp.concatenate(rows, axis=0))

            qkv = [None] * G
            sc = [None] * G
            p = [None] * G
            o = [None] * G
            acc = None
            for it in range(G + WO_LAG):
                if it < G:
                    qkv[it] = (proj(wq_s, it), proj(wk_s, it), proj(wv_s, it))
                if 0 <= it - 1 < G:
                    sc[it - 1] = scores(qkv[it - 1][0], qkv[it - 1][1])
                if 0 <= it - 2 < G:
                    o[it - 2] = pv(p[it - 2], qkv[it - 2][2])
                if 0 <= it - 1 < G:
                    p[it - 1] = softmax(sc[it - 1])
                if 0 <= it - WO_LAG < G:
                    t = out_proj(it - WO_LAG, o[it - WO_LAG])
                    acc = t if acc is None else acc + t
            xs_ref[r, :] = xs_ref[r, :] + acc[M:, :]
            return acc[:M, :]

        def b_pass1(t, _):
            r0 = pl.multiple_of(t * RT, RT)
            xl = _ln(xs_ref[pl.ds(r0, RT), :])
            ln_ref[pl.ds(r0, RT), :] = xl
            h = _gelu(_dot(_ln(xl).astype(BF16), w1_ref[...]))
            h_ref[pl.ds(r0 + HALO, RT), :] = h
            return 0

        def b_pass2(t, last):
            r0 = pl.multiple_of(t * RT, RT)
            pieces = []
            shifts = (-1, 1, -2, 2)
            for lt in range(D // 128):
                c0 = lt * 128
                win = h_ref[pl.ds(r0, RT + 2 * HALO), pl.ds(c0, 128)]
                g_lo, g_hi = c0 // c, min((c0 + 127) // c, 3)
                a = win[HALO + shifts[g_lo]: HALO + shifts[g_lo] + RT]
                if g_hi != g_lo:
                    b = win[HALO + shifts[g_hi]: HALO + shifts[g_hi] + RT]
                    lane = jax.lax.broadcasted_iota(I32, (RT, 128), 1) + c0
                    a = jnp.where(lane < g_hi * c, a, b)
                pieces.append(a)
            hs_in = jnp.concatenate(pieces, axis=1).astype(BF16)
            x1 = ln_ref[pl.ds(r0, RT), :] + _dot(hs_in, w2_ref[...])
            g = _gelu(_dot(_ln(x1).astype(BF16), w3_ref[...]))
            h2 = _dot(g.astype(BF16), w4_ref[...])
            xn = xs_ref[pl.ds(r0, RT), :] + (x1 + h2)
            if last:
                out_ref[pl.ds(r0, RT), :] = xn.astype(out_ref.dtype)
            else:
                xs_ref[pl.ds(r0, RT), :] = xn
                ln_ref[pl.ds(r0, RT), :] = _ln(xn)
            return 0

        for layer in range(2):
            last = layer == 1
            with jax.named_scope('A%d' % layer):
                jax.lax.fori_loop(0, NSEG, a_step, mem0_ref[...].astype(F32))
            if layer == 0:
                for cp in w_cps[1:]:
                    cp.wait()
            with jax.named_scope('Bp1_%d' % layer):
                jax.lax.fori_loop(0, NT, b_pass1, 0)
            with jax.named_scope('Bp2_%d' % layer):
                jax.lax.fori_loop(0, NT, functools.partial(_b2_body, b_pass2, last), 0)

    return kernel


def _b2_body(fn, last, t, carry):
    return fn(t, last)


@functools.partial(jax.jit, static_argnames=("A_seg_len",))
def pallas_interleave_layers__memory_aug_recurrent_mem_tr__mixer_s_mlp__prompt_kernel(
    A_x: jax.Array,
    A_mem0: jax.Array,
    A_Wq: jax.Array,
    A_Wk: jax.Array,
    A_Wv: jax.Array,
    A_Wo: jax.Array,
    A_seg_len,
    B_x: jax.Array,
    B_w1: jax.Array,
    B_w2: jax.Array,
    B_w3: jax.Array,
    B_w4: jax.Array,
):
    del B_x
    B, S, D = A_x.shape
    assert B == 1
    H, Dh = A_Wq.shape[1], A_Wq.shape[2]
    M = A_mem0.shape[1]
    SEG = int(A_seg_len)
    F = B_w3.shape[1]
    kernel = _make_kernel(S, D, H, Dh, M, SEG, F)
    hbm = pl.BlockSpec(memory_space=pl.ANY)
    nt = 3 * H // 2

    def wt(w):
        return jnp.transpose(w, (1, 2, 0)).reshape(H * Dh, D)

    out = pl.pallas_call(
        kernel,
        out_shape=jax.ShapeDtypeStruct((S, D), A_x.dtype),
        in_specs=[pl.BlockSpec()] + [hbm] * 9,
        scratch_shapes=[
            pltpu.VMEM((S, D), BF16),
            pltpu.VMEM((3, H * Dh, D), BF16),
            pltpu.VMEM((nt, D // 2, 128), I32),
            pltpu.VMEM((nt, D // 2, 128), I32),
            pltpu.VMEM((nt, D // 2, 128), I32),
            pltpu.VMEM((H * Dh, D), BF16),
            pltpu.VMEM((D, D), BF16),
            pltpu.VMEM((D, D), BF16),
            pltpu.VMEM((D, F), BF16),
            pltpu.VMEM((F, D), BF16),
            pltpu.VMEM((S, D), F32),
            pltpu.VMEM((S, D), F32),
            pltpu.VMEM((S + 16, D), F32),
            pltpu.SemaphoreType.DMA((1,)),
            pltpu.SemaphoreType.DMA((24,)),
            pltpu.SemaphoreType.DMA((5,)),
        ],
        compiler_params=pltpu.CompilerParams(vmem_limit_bytes=110 * 1024 * 1024),
    )(
        A_mem0.reshape(M, D), A_x.reshape(S, D), wt(A_Wq), wt(A_Wk), wt(A_Wv),
        A_Wo.reshape(H * Dh, D), B_w1, B_w2, B_w3, B_w4,
    )
    return out.reshape(B, S, D)
```

```python
import functools

import jax
import jax.numpy as jnp
import numpy as np
import jax.experimental.pallas as pl
import jax.experimental.pallas.tpu as pltpu

F32 = jnp.float32
BF16 = jnp.bfloat16
I32 = jnp.int32
_NEG = -1000000000.0


def _ln(x, eps=1e-05):
    m = jnp.mean(x, axis=-1, keepdims=True)
    d = x - m
    v = jnp.mean(d * d, axis=-1, keepdims=True)
    return d * jax.lax.rsqrt(v + eps)


def _gelu(x):
    c = float(np.sqrt(2.0 / np.pi))
    return 0.5 * x * (1.0 + jnp.tanh(c * (x + 0.044715 * (x * x * x))))


def _dot(a, b):
    return jnp.dot(a, b, preferred_element_type=F32)


def _dot_nt(a, b):
    return jax.lax.dot_general(a, b, (((1,), (1,)), ((), ())), preferred_element_type=F32)


def _make_kernel(S, D, H, Dh, M, SEG, F, G=8, WO_LAG=4, AHEAD=4):
    L = M + SEG
    NSEG = S // SEG
    NP = H // 2
    PP = NP // G
    scale = Dh ** (-0.5)
    RT = 256
    NT = S // RT
    HALO = 8
    c = D // 4
    GR = PP * 2 * Dh
    assert Dh == 192 and D % 128 == 0

    def kernel(mem0_ref, x_hbm, wq_hbm, wk_hbm, wv_hbm, wo_hbm,
               w1_hbm, w2_hbm, w3_hbm, w4_hbm, out_hbm,
               x_v, stage, wq_s, wk_s, wv_s, wo_ref, w1_ref, w2_ref, w3_ref, w4_ref,
               xs_ref, ln_ref, xl_ref, h_ref, sem_x, sem_st, sem_w, sem_o):
        def st_copy(g, mi):
            rows = pl.ds(g * GR, GR)
            return pltpu.make_async_copy(
                (wq_hbm, wk_hbm, wv_hbm)[mi].at[rows], stage.at[mi, rows], sem_st.at[3 * g + mi])

        cp_x = pltpu.make_async_copy(x_hbm, x_v, sem_x.at[0])
        w_cps = [pltpu.make_async_copy(src, dst, sem_w.at[wi])
                 for wi, (src, dst) in enumerate(
                     ((wo_hbm, wo_ref), (w1_hbm, w1_ref), (w2_hbm, w2_ref),
                      (w3_hbm, w3_ref), (w4_hbm, w4_ref)))]
        dmas = [st_copy(g, mi) for g in range(G) for mi in range(3)] + [cp_x, w_cps[0]]
        for cp in dmas[:AHEAD]:
            cp.start()

        for i in range(3 * G):
            g, mi = divmod(i, 3)
            dst = (wq_s, wk_s, wv_s)[mi]
            dmas[i].wait()
            if i + AHEAD < len(dmas):
                dmas[i + AHEAD].start()

            def relayout(u, _, mi=mi, g=g, dst=dst):
                j = g * PP + u
                r0 = pl.multiple_of(j * 2 * Dh, 128)
                a = stage[mi, pl.ds(r0, 128), :]
                b = stage[mi, pl.ds(r0 + Dh, 128), :]
                t = jnp.concatenate([stage[mi, pl.ds(r0 + 128, 64), :],
                                     stage[mi, pl.ds(r0 + Dh + 128, 64), :]], axis=0)
                for n, v in enumerate((a, b, t)):
                    dst[3 * j + n] = pltpu.bitcast(v.T, I32)
                return 0
            jax.lax.fori_loop(0, PP, relayout, 0)
        for cp in dmas[3 * G + AHEAD:]:
            cp.start()

        cp_x.wait()

        def init_tile(t, _):
            r = pl.ds(pl.multiple_of(t * RT, RT), RT)
            x = x_v[r, :].astype(F32)
            xs_ref[r, :] = x
            ln_ref[r, :] = _ln(x)
            return 0
        jax.lax.fori_loop(0, NT, init_tile, 0)
        h_ref[pl.ds(0, HALO), :] = jnp.zeros((HALO, D), F32)
        h_ref[pl.ds(HALO + S, HALO), :] = jnp.zeros((HALO, D), F32)
        w_cps[0].wait()
        for cp in w_cps[1:]:
            cp.start()

        def a_step(s, mem):
            r = pl.ds(pl.multiple_of(s * SEG, SEG), SEG)
            hrows = jnp.concatenate([mem, ln_ref[r, :]], axis=0)
            lo64 = jax.lax.broadcasted_iota(I32, (L, 128), 1) < 64
            zero = jnp.zeros((L, 128), F32)
            rowb = jax.lax.broadcasted_iota(I32, (PP * L, 2 * L), 0) % L
            colb = jax.lax.broadcasted_iota(I32, (PP * L, 2 * L), 1)
            lob = colb < L
            maskb = (rowb < M) | (rowb >= jnp.where(lob, colb, colb - L))

            def proj(w_s, g):
                w = jnp.concatenate(
                    [pltpu.bitcast(w_s[3 * PP * g + t], BF16) for t in range(3 * PP)], axis=1)
                return _dot(hrows, w)

            def stack(x, j):
                t0 = x[:, 384 * j:384 * j + 128]
                t1 = x[:, 384 * j + 128:384 * j + 256]
                t2 = x[:, 384 * j + 256:384 * j + 384]
                top = jnp.concatenate([t0, zero, jnp.where(lo64, t2, 0.0)], axis=1)
                bot = jnp.concatenate([zero, t1, jnp.where(lo64, 0.0, t2)], axis=1)
                return jnp.concatenate([top, bot], axis=0).astype(BF16)

            def scores(q, k):
                return jnp.concatenate(
                    [_dot_nt(q[:, 384 * j:384 * (j + 1)], stack(k, j)) for j in range(PP)],
                    axis=0) * scale

            def softmax(sc):
                sc = jnp.where(maskb, sc, _NEG)
                m_lo = jnp.max(jnp.where(lob, sc, -jnp.inf), axis=1, keepdims=True)
                m_hi = jnp.max(jnp.where(lob, -jnp.inf, sc), axis=1, keepdims=True)
                e = jnp.exp(sc - jnp.where(lob, m_lo, m_hi))
                s_lo = jnp.sum(jnp.where(lob, e, 0.0), axis=1, keepdims=True)
                s_hi = jnp.sum(jnp.where(lob, 0.0, e), axis=1, keepdims=True)
                return e / jnp.where(lob, s_lo, s_hi)

            def pv(p, v):
                return jnp.concatenate(
                    [_dot(p[j * L:(j + 1) * L], stack(v, j)) for j in range(PP)], axis=1)

            def out_proj(g, o):
                rows = []
                for j in range(PP):
                    r0 = (g * PP + j) * 2 * Dh
                    rows += [wo_ref[r0:r0 + 128, :], wo_ref[r0 + Dh:r0 + Dh + 128, :],
                             wo_ref[r0 + 128:r0 + Dh, :], wo_ref[r0 + Dh + 128:r0 + 2 * Dh, :]]
                return _dot(o, jnp.concatenate(rows, axis=0))

            qkv = [None] * G
            sc = [None] * G
            p = [None] * G
            o = [None] * G
            acc = None
            for it in range(G + WO_LAG):
                if it < G:
                    qkv[it] = (proj(wq_s, it), proj(wk_s, it), proj(wv_s, it))
                if 0 <= it - 1 < G:
                    sc[it - 1] = scores(qkv[it - 1][0], qkv[it - 1][1])
                if 0 <= it - 2 < G:
                    o[it - 2] = pv(p[it - 2], qkv[it - 2][2])
                if 0 <= it - 1 < G:
                    p[it - 1] = softmax(sc[it - 1])
                if 0 <= it - WO_LAG < G:
                    t = out_proj(it - WO_LAG, o[it - WO_LAG])
                    acc = t if acc is None else acc + t
            xs_ref[r, :] = xs_ref[r, :] + acc[M:, :]
            return acc[:M, :]

        def b1_in(t):
            return xs_ref[pl.ds(pl.multiple_of(t * RT, RT), RT), :]

        def b1_mid(t, x):
            xl = _ln(x)
            xl_ref[pl.ds(pl.multiple_of(t * RT, RT), RT), :] = xl
            return _dot(_ln(xl).astype(BF16), w1_ref[...])

        def b1_out(t, h1):
            h_ref[pl.ds(pl.multiple_of(t * RT, RT) + HALO, RT), :] = _gelu(h1)

        def b2_in(t):
            r0 = pl.multiple_of(t * RT, RT)
            pieces = []
            shifts = (-1, 1, -2, 2)
            for lt in range(D // 128):
                c0 = lt * 128
                win = h_ref[pl.ds(r0, RT + 2 * HALO), pl.ds(c0, 128)]
                g_lo, g_hi = c0 // c, min((c0 + 127) // c, 3)
                a = win[HALO + shifts[g_lo]: HALO + shifts[g_lo] + RT]
                if g_hi != g_lo:
                    bb = win[HALO + shifts[g_hi]: HALO + shifts[g_hi] + RT]
                    lane = jax.lax.broadcasted_iota(I32, (RT, 128), 1) + c0
                    a = jnp.where(lane < g_hi * c, a, bb)
                pieces.append(a)
            hs_in = jnp.concatenate(pieces, axis=1).astype(BF16)
            return hs_in, xl_ref[pl.ds(r0, RT), :], xs_ref[pl.ds(r0, RT), :]

        def b_tile(t, ahead, last):
            r = pl.ds(pl.multiple_of(t * RT, RT), RT)
            hs_in, xl_t, x_t = b2_in(t)
            if ahead:
                x_n = b1_in(t + 2)
            x1 = xl_t + _dot(hs_in, w2_ref[...])
            if ahead:
                h1 = b1_mid(t + 2, x_n)
            g = _gelu(_dot(_ln(x1).astype(BF16), w3_ref[...]))
            if ahead:
                b1_out(t + 2, h1)
            xn = x_t + (x1 + _dot(g.astype(BF16), w4_ref[...]))
            if last:
                x_v[r, :] = xn.astype(BF16)
                out_copy(t).start()
            else:
                xs_ref[r, :] = xn
                ln_ref[r, :] = _ln(xn)

        def out_copy(t):
            r = pl.ds(pl.multiple_of(t * RT, RT), RT)
            return pltpu.make_async_copy(x_v.at[r], out_hbm.at[r], sem_o.at[t])

        def b1_tile(t, _):
            b1_out(t, b1_mid(t, b1_in(t)))
            return 0

        for layer in range(2):
            last = layer == 1
            with jax.named_scope('A%d' % layer):
                jax.lax.fori_loop(0, NSEG, a_step, mem0_ref[...].astype(F32))
            if layer == 0:
                for cp in w_cps[1:]:
                    cp.wait()
            with jax.named_scope('Bp1_%d' % layer):
                jax.lax.fori_loop(0, 2, b1_tile, 0)
            with jax.named_scope('Bp2_%d' % layer):
                jax.lax.fori_loop(0, NT - 2, functools.partial(_b_body, b_tile, True, last), 0)
            with jax.named_scope('Bp3_%d' % layer):
                jax.lax.fori_loop(NT - 2, NT, functools.partial(_b_body, b_tile, False, last), 0)
        for t in range(NT):
            out_copy(t).wait()

    return kernel


def _b_body(fn, ahead, last, t, carry):
    fn(t, ahead, last)
    return carry


@functools.partial(jax.jit, static_argnames=("A_seg_len",))
def pallas_interleave_layers__memory_aug_recurrent_mem_tr__mixer_s_mlp__prompt_kernel(
    A_x: jax.Array,
    A_mem0: jax.Array,
    A_Wq: jax.Array,
    A_Wk: jax.Array,
    A_Wv: jax.Array,
    A_Wo: jax.Array,
    A_seg_len,
    B_x: jax.Array,
    B_w1: jax.Array,
    B_w2: jax.Array,
    B_w3: jax.Array,
    B_w4: jax.Array,
):
    del B_x
    B, S, D = A_x.shape
    assert B == 1
    H, Dh = A_Wq.shape[1], A_Wq.shape[2]
    M = A_mem0.shape[1]
    SEG = int(A_seg_len)
    F = B_w3.shape[1]
    kernel = _make_kernel(S, D, H, Dh, M, SEG, F)
    hbm = pl.BlockSpec(memory_space=pl.ANY)
    nt = 3 * H // 2

    def wt(w):
        return jnp.transpose(w, (1, 2, 0)).reshape(H * Dh, D)

    out = pl.pallas_call(
        kernel,
        out_shape=jax.ShapeDtypeStruct((S, D), A_x.dtype),
        in_specs=[pl.BlockSpec()] + [hbm] * 9,
        out_specs=hbm,
        scratch_shapes=[
            pltpu.VMEM((S, D), BF16),
            pltpu.VMEM((3, H * Dh, D), BF16),
            pltpu.VMEM((nt, D // 2, 128), I32),
            pltpu.VMEM((nt, D // 2, 128), I32),
            pltpu.VMEM((nt, D // 2, 128), I32),
            pltpu.VMEM((H * Dh, D), BF16),
            pltpu.VMEM((D, D), BF16),
            pltpu.VMEM((D, D), BF16),
            pltpu.VMEM((D, F), BF16),
            pltpu.VMEM((F, D), BF16),
            pltpu.VMEM((S, D), F32),
            pltpu.VMEM((S, D), F32),
            pltpu.VMEM((S, D), F32),
            pltpu.VMEM((S + 16, D), F32),
            pltpu.SemaphoreType.DMA((1,)),
            pltpu.SemaphoreType.DMA((24,)),
            pltpu.SemaphoreType.DMA((5,)),
            pltpu.SemaphoreType.DMA((8,)),
        ],
        compiler_params=pltpu.CompilerParams(vmem_limit_bytes=110 * 1024 * 1024),
    )(
        A_mem0.reshape(M, D), A_x.reshape(S, D), wt(A_Wq), wt(A_Wk), wt(A_Wv),
        A_Wo.reshape(H * Dh, D), B_w1, B_w2, B_w3, B_w4,
    )
    return out.reshape(B, S, D)
```

```python
import functools

import jax
import jax.numpy as jnp
import numpy as np
import jax.experimental.pallas as pl
import jax.experimental.pallas.tpu as pltpu

F32 = jnp.float32
BF16 = jnp.bfloat16
I32 = jnp.int32
_NEG = -1000000000.0


def _ln(x, eps=1e-05):
    m = jnp.mean(x, axis=-1, keepdims=True)
    d = x - m
    v = jnp.mean(d * d, axis=-1, keepdims=True)
    return d * jax.lax.rsqrt(v + eps)


def _gelu(x):
    c = float(np.sqrt(2.0 / np.pi))
    return 0.5 * x * (1.0 + jnp.tanh(c * (x + 0.044715 * (x * x * x))))


def _dot(a, b):
    return jnp.dot(a, b, preferred_element_type=F32)


def _dot_nt(a, b):
    return jax.lax.dot_general(a, b, (((1,), (1,)), ((), ())), preferred_element_type=F32)


def _make_kernel(S, D, H, Dh, M, SEG, F, G=8, WO_LAG=4, RAMP=3):
    L = M + SEG
    NSEG = S // SEG
    NP = H // 2
    PP = NP // G
    scale = Dh ** (-0.5)
    RT = 256
    NT = S // RT
    HALO = 8
    c = D // 4
    PW = 2 * Dh
    AHEAD = RAMP + 1
    XR = 24
    LEAD = 12 * XR
    NLEAD = LEAD // (SEG - XR)
    RING = 384
    X0 = LEAD
    IT = 160
    assert Dh == 192 and D % 128 == 0
    assert RING % XR == 0 and RING % SEG == 0 and (S - X0) % IT == 0 and RING >= LEAD + XR

    def kernel(mem0_ref, x_hbm, wq_hbm, wk_hbm, wv_hbm, wo_hbm,
               w1_hbm, w2_hbm, w3_hbm, w4_hbm, out_hbm,
               x_v, stage, wq_s, wk_s, wv_s, wo_ref, w1_ref, w2_ref, w3_ref, w4_ref,
               xs_ref, ln_ref, xl_ref, h_ref, ring, sem_x, sem_st, sem_w, sem_o):
        def st_copy(j, mi):
            rows = pl.ds(pl.multiple_of(j * PW, 128), PW)
            return pltpu.make_async_copy(
                (wq_hbm, wk_hbm, wv_hbm)[mi].at[rows], stage.at[mi, rows], sem_st.at[3 * j + mi])

        cp_x0 = pltpu.make_async_copy(x_hbm.at[pl.ds(0, X0)], x_v.at[pl.ds(0, X0)], sem_x.at[0])
        cp_x1 = pltpu.make_async_copy(
            x_hbm.at[pl.ds(X0, S - X0)], x_v.at[pl.ds(X0, S - X0)], sem_x.at[1])
        w_cps = [pltpu.make_async_copy(src, dst, sem_w.at[wi])
                 for wi, (src, dst) in enumerate(
                     ((wo_hbm, wo_ref), (w1_hbm, w1_ref), (w2_hbm, w2_ref),
                      (w3_hbm, w3_ref), (w4_hbm, w4_ref)))]
        cp_x0.start()
        for j in range(2):
            for mi in range(3):
                st_copy(j, mi).start()

        def prenorm(r):
            x = x_v[r, :].astype(F32)
            xs_ref[r, :] = x
            ln_ref[r, :] = _ln(x)

        cp_x0.wait()
        prenorm(pl.ds(0, X0))
        h_ref[pl.ds(0, HALO), :] = jnp.zeros((HALO, D), F32)
        h_ref[pl.ds(HALO + S, HALO), :] = jnp.zeros((HALO, D), F32)

        def relayout(j):
            r0 = pl.multiple_of(j * PW, 128)
            for mi, dst in enumerate((wq_s, wk_s, wv_s)):
                a = stage[mi, pl.ds(r0, 128), :]
                b = stage[mi, pl.ds(r0 + Dh, 128), :]
                t = jnp.concatenate([stage[mi, pl.ds(r0 + 128, 64), :],
                                     stage[mi, pl.ds(r0 + Dh + 128, 64), :]], axis=0)
                for n, v in enumerate((a, b, t)):
                    dst[3 * j + n] = pltpu.bitcast(v.T, I32)

        def pair_w(w_s, j):
            return jnp.concatenate(
                [pltpu.bitcast(w_s[3 * j + t], BF16) for t in range(3)], axis=1)

        def lead_proj(j):
            rows = ln_ref[pl.ds(0, LEAD), :]
            for mi, w_s in enumerate((wq_s, wk_s, wv_s)):
                ring[mi, j, pl.ds(0, LEAD), :] = _dot(rows, pair_w(w_s, j))

        def arrive(j):
            for mi in range(3):
                st_copy(j, mi).wait()

            @pl.when(j + AHEAD < NP)
            def _():
                for mi in range(3):
                    st_copy(j + AHEAD, mi).start()

            @pl.when(j + AHEAD == NP)
            def _():
                cp_x1.start()
                w_cps[0].start()

        for j in range(2, RAMP + 1):
            for mi in range(3):
                st_copy(j - 2, mi).wait()
                st_copy(2 * j - 2, mi).start()
                st_copy(2 * j - 1, mi).start()
            relayout(j - 2)
            if j > 2:
                lead_proj(j - 3)

        def startup(j, _):
            arrive(j)
            lead_proj(j - 1)
            relayout(j)
            return 0
        with jax.named_scope('startup'):
            jax.lax.fori_loop(RAMP - 1, NP, startup, 0)
            lead_proj(NP - 1)
        cp_x1.wait()

        def init_tile(t, _):
            prenorm(pl.ds(pl.multiple_of(X0 + t * IT, 8), IT))
            return 0
        jax.lax.fori_loop(0, (S - X0) // IT, init_tile, 0)
        with jax.named_scope('wait_wo'):
            w_cps[0].wait()
        for cp in w_cps[1:]:
            cp.start()

        def a_step(lead, s, mem):
            r = pl.ds(pl.multiple_of(s * SEG, SEG), SEG)
            if lead:
                p0 = LEAD + s * XR
                hrows = jnp.concatenate([mem, ln_ref[pl.ds(pl.multiple_of(p0, 8), XR), :]], axis=0)
                wpos = pl.ds(pl.multiple_of(jax.lax.rem(p0, RING), 8), XR)
                rpos = pl.ds(pl.multiple_of(jax.lax.rem(s * SEG, RING), 8), SEG)
            else:
                hrows = jnp.concatenate([mem, ln_ref[r, :]], axis=0)
            lo64 = jax.lax.broadcasted_iota(I32, (L, 128), 1) < 64
            zero = jnp.zeros((L, 128), F32)
            rowb = jax.lax.broadcasted_iota(I32, (PP * L, 2 * L), 0) % L
            colb = jax.lax.broadcasted_iota(I32, (PP * L, 2 * L), 1)
            lob = colb < L
            maskb = (rowb < M) | (rowb >= jnp.where(lob, colb, colb - L))

            def proj(mi, g):
                w_s = (wq_s, wk_s, wv_s)[mi]
                y = _dot(hrows, jnp.concatenate(
                    [pair_w(w_s, g * PP + u) for u in range(PP)], axis=1))
                if lead:
                    for u in range(PP):
                        ring[mi, g * PP + u, wpos, :] = y[M:, u * PW:(u + 1) * PW]
                    y = jnp.concatenate([y[:M, :], jnp.concatenate(
                        [ring[mi, g * PP + u, rpos, :] for u in range(PP)], axis=1)], axis=0)
                return y

            def stack(x, j):
                t0 = x[:, 384 * j:384 * j + 128]
                t1 = x[:, 384 * j + 128:384 * j + 256]
                t2 = x[:, 384 * j + 256:384 * j + 384]
                top = jnp.concatenate([t0, zero, jnp.where(lo64, t2, 0.0)], axis=1)
                bot = jnp.concatenate([zero, t1, jnp.where(lo64, 0.0, t2)], axis=1)
                return jnp.concatenate([top, bot], axis=0).astype(BF16)

            def scores(q, k):
                return jnp.concatenate(
                    [_dot_nt(q[:, 384 * j:384 * (j + 1)], stack(k, j)) for j in range(PP)],
                    axis=0) * scale

            def softmax(sc):
                sc = jnp.where(maskb, sc, _NEG)
                m_lo = jnp.max(jnp.where(lob, sc, -jnp.inf), axis=1, keepdims=True)
                m_hi = jnp.max(jnp.where(lob, -jnp.inf, sc), axis=1, keepdims=True)
                e = jnp.exp(sc - jnp.where(lob, m_lo, m_hi))
                s_lo = jnp.sum(jnp.where(lob, e, 0.0), axis=1, keepdims=True)
                s_hi = jnp.sum(jnp.where(lob, 0.0, e), axis=1, keepdims=True)
                return e / jnp.where(lob, s_lo, s_hi)

            def pv(p, v):
                return jnp.concatenate(
                    [_dot(p[j * L:(j + 1) * L], stack(v, j)) for j in range(PP)], axis=1)

            def out_proj(g, o):
                rows = []
                for j in range(PP):
                    r0 = (g * PP + j) * 2 * Dh
                    rows += [wo_ref[r0:r0 + 128, :], wo_ref[r0 + Dh:r0 + Dh + 128, :],
                             wo_ref[r0 + 128:r0 + Dh, :], wo_ref[r0 + Dh + 128:r0 + 2 * Dh, :]]
                return _dot(o, jnp.concatenate(rows, axis=0))

            qkv = [None] * G
            sc = [None] * G
            p = [None] * G
            o = [None] * G
            acc = None
            for it in range(G + WO_LAG):
                if it < G:
                    qkv[it] = (proj(0, it), proj(1, it), proj(2, it))
                if 0 <= it - 1 < G:
                    sc[it - 1] = scores(qkv[it - 1][0], qkv[it - 1][1])
                if 0 <= it - 2 < G:
                    o[it - 2] = pv(p[it - 2], qkv[it - 2][2])
                if 0 <= it - 1 < G:
                    p[it - 1] = softmax(sc[it - 1])
                if 0 <= it - WO_LAG < G:
                    t = out_proj(it - WO_LAG, o[it - WO_LAG])
                    acc = t if acc is None else acc + t
            xs_ref[r, :] = xs_ref[r, :] + acc[M:, :]
            return acc[:M, :]

        def b1_in(t):
            return xs_ref[pl.ds(pl.multiple_of(t * RT, RT), RT), :]

        def b1_mid(t, x):
            xl = _ln(x)
            xl_ref[pl.ds(pl.multiple_of(t * RT, RT), RT), :] = xl
            return _dot(_ln(xl).astype(BF16), w1_ref[...])

        def b1_out(t, h1):
            h_ref[pl.ds(pl.multiple_of(t * RT, RT) + HALO, RT), :] = _gelu(h1)

        def b2_in(t):
            r0 = pl.multiple_of(t * RT, RT)
            pieces = []
            shifts = (-1, 1, -2, 2)
            for lt in range(D // 128):
                c0 = lt * 128
                win = h_ref[pl.ds(r0, RT + 2 * HALO), pl.ds(c0, 128)]
                g_lo, g_hi = c0 // c, min((c0 + 127) // c, 3)
                a = win[HALO + shifts[g_lo]: HALO + shifts[g_lo] + RT]
                if g_hi != g_lo:
                    bb = win[HALO + shifts[g_hi]: HALO + shifts[g_hi] + RT]
                    lane = jax.lax.broadcasted_iota(I32, (RT, 128), 1) + c0
                    a = jnp.where(lane < g_hi * c, a, bb)
                pieces.append(a)
            hs_in = jnp.concatenate(pieces, axis=1).astype(BF16)
            return hs_in, xl_ref[pl.ds(r0, RT), :], xs_ref[pl.ds(r0, RT), :]

        def b_tile(t, ahead, last):
            r = pl.ds(pl.multiple_of(t * RT, RT), RT)
            hs_in, xl_t, x_t = b2_in(t)
            if ahead:
                x_n = b1_in(t + 2)
            x1 = xl_t + _dot(hs_in, w2_ref[...])
            if ahead:
                h1 = b1_mid(t + 2, x_n)
            g = _gelu(_dot(_ln(x1).astype(BF16), w3_ref[...]))
            if ahead:
                b1_out(t + 2, h1)
            xn = x_t + (x1 + _dot(g.astype(BF16), w4_ref[...]))
            if last:
                x_v[r, :] = xn.astype(BF16)
                out_copy(t).start()
            else:
                xs_ref[r, :] = xn
                ln_ref[r, :] = _ln(xn)

        def out_copy(t):
            r = pl.ds(pl.multiple_of(t * RT, RT), RT)
            return pltpu.make_async_copy(x_v.at[r], out_hbm.at[r], sem_o.at[t])

        def b1_tile(t, _):
            b1_out(t, b1_mid(t, b1_in(t)))
            return 0

        for layer in range(2):
            last = layer == 1
            with jax.named_scope('A%d' % layer):
                mem = mem0_ref[...].astype(F32)
                if layer == 0:
                    mem = jax.lax.fori_loop(0, NLEAD, functools.partial(a_step, True), mem)
                jax.lax.fori_loop(NLEAD if layer == 0 else 0, NSEG,
                                  functools.partial(a_step, False), mem)
            if layer == 0:
                for cp in w_cps[1:]:
                    cp.wait()
            with jax.named_scope('Bp1_%d' % layer):
                jax.lax.fori_loop(0, 2, b1_tile, 0)
            with jax.named_scope('Bp2_%d' % layer):
                jax.lax.fori_loop(0, NT - 2, functools.partial(_b_body, b_tile, True, last), 0)
            with jax.named_scope('Bp3_%d' % layer):
                jax.lax.fori_loop(NT - 2, NT, functools.partial(_b_body, b_tile, False, last), 0)
        for t in range(NT):
            out_copy(t).wait()

    return kernel


def _b_body(fn, ahead, last, t, carry):
    fn(t, ahead, last)
    return carry


@functools.partial(jax.jit, static_argnames=("A_seg_len",))
def pallas_interleave_layers__memory_aug_recurrent_mem_tr__mixer_s_mlp__prompt_kernel(
    A_x: jax.Array,
    A_mem0: jax.Array,
    A_Wq: jax.Array,
    A_Wk: jax.Array,
    A_Wv: jax.Array,
    A_Wo: jax.Array,
    A_seg_len,
    B_x: jax.Array,
    B_w1: jax.Array,
    B_w2: jax.Array,
    B_w3: jax.Array,
    B_w4: jax.Array,
):
    del B_x
    B, S, D = A_x.shape
    assert B == 1
    H, Dh = A_Wq.shape[1], A_Wq.shape[2]
    M = A_mem0.shape[1]
    SEG = int(A_seg_len)
    F = B_w3.shape[1]
    kernel = _make_kernel(S, D, H, Dh, M, SEG, F)
    hbm = pl.BlockSpec(memory_space=pl.ANY)
    nt = 3 * H // 2

    def wt(w):
        return jnp.transpose(w, (1, 2, 0)).reshape(H * Dh, D)

    out = pl.pallas_call(
        kernel,
        out_shape=jax.ShapeDtypeStruct((S, D), A_x.dtype),
        in_specs=[pl.BlockSpec()] + [hbm] * 9,
        out_specs=hbm,
        scratch_shapes=[
            pltpu.VMEM((S, D), BF16),
            pltpu.VMEM((3, H * Dh, D), BF16),
            pltpu.VMEM((nt, D // 2, 128), I32),
            pltpu.VMEM((nt, D // 2, 128), I32),
            pltpu.VMEM((nt, D // 2, 128), I32),
            pltpu.VMEM((H * Dh, D), BF16),
            pltpu.VMEM((D, D), BF16),
            pltpu.VMEM((D, D), BF16),
            pltpu.VMEM((D, F), BF16),
            pltpu.VMEM((F, D), BF16),
            pltpu.VMEM((S, D), F32),
            pltpu.VMEM((S, D), F32),
            pltpu.VMEM((S, D), F32),
            pltpu.VMEM((S + 16, D), F32),
            pltpu.VMEM((3, 16, 384, 384), F32),
            pltpu.SemaphoreType.DMA((2,)),
            pltpu.SemaphoreType.DMA((48,)),
            pltpu.SemaphoreType.DMA((5,)),
            pltpu.SemaphoreType.DMA((8,)),
        ],
        compiler_params=pltpu.CompilerParams(vmem_limit_bytes=120 * 1024 * 1024),
    )(
        A_mem0.reshape(M, D), A_x.reshape(S, D), wt(A_Wq), wt(A_Wk), wt(A_Wv),
        A_Wo.reshape(H * Dh, D), B_w1, B_w2, B_w3, B_w4,
    )
    return out.reshape(B, S, D)
```

```python
import functools

import jax
import jax.numpy as jnp
import numpy as np
import jax.experimental.pallas as pl
import jax.experimental.pallas.tpu as pltpu

F32 = jnp.float32
BF16 = jnp.bfloat16
I32 = jnp.int32
_NEG = -1000000000.0


def _ln(x, eps=1e-05):
    m = jnp.mean(x, axis=-1, keepdims=True)
    d = x - m
    v = jnp.mean(d * d, axis=-1, keepdims=True)
    return d * jax.lax.rsqrt(v + eps)


def _gelu(x):
    c = float(np.sqrt(2.0 / np.pi))
    return 0.5 * x * (1.0 + jnp.tanh(c * (x + 0.044715 * (x * x * x))))


def _dot(a, b):
    return jnp.dot(a, b, preferred_element_type=F32)


def _dot_nt(a, b):
    return jax.lax.dot_general(a, b, (((1,), (1,)), ((), ())), preferred_element_type=F32)


def _make_kernel(S, D, H, Dh, M, SEG, F, G=8, WO_LAG=4, RAMP=4, UNR=2):
    L = M + SEG
    NSEG = S // SEG
    NP = H // 2
    PP = NP // G
    scale = Dh ** (-0.5)
    RT = 256
    NT = S // RT
    HALO = 8
    c = D // 4
    PW = 2 * Dh
    AHEAD = RAMP + 1
    XR = 24
    LEAD = 12 * XR
    NLEAD = LEAD // (SEG - XR)
    RING = 384
    X0 = LEAD
    IT = 160
    assert Dh == 192 and D % 128 == 0
    assert RING % XR == 0 and RING % SEG == 0 and (S - X0) % IT == 0 and RING >= LEAD + XR

    def kernel(mem0_hbm, x_hbm, wq_hbm, wk_hbm, wv_hbm, wo_hbm,
               w1_hbm, w2_hbm, w3_hbm, w4_hbm, out_hbm,
               x_v, stage, wq_s, wk_s, wv_s, wo_ref, w1_ref, w2_ref, w3_ref, w4_ref,
               xs_ref, ln_ref, xl_ref, h_ref, ring, mem0_ref, sem_x, sem_st, sem_w, sem_o):
        def st_copy(j, mi):
            rows = pl.ds(pl.multiple_of(j * PW, 128), PW)
            return pltpu.make_async_copy(
                (wq_hbm, wk_hbm, wv_hbm)[mi].at[rows], stage.at[mi, rows], sem_st.at[3 * j + mi])

        cp_x0 = pltpu.make_async_copy(x_hbm.at[pl.ds(0, X0)], x_v.at[pl.ds(0, X0)], sem_x.at[0])
        cp_x1 = pltpu.make_async_copy(
            x_hbm.at[pl.ds(X0, S - X0)], x_v.at[pl.ds(X0, S - X0)], sem_x.at[1])
        w_cps = [pltpu.make_async_copy(src, dst, sem_w.at[wi])
                 for wi, (src, dst) in enumerate(
                     ((wo_hbm, wo_ref), (w1_hbm, w1_ref), (w2_hbm, w2_ref),
                      (w3_hbm, w3_ref), (w4_hbm, w4_ref)))]
        cp_x0.start()
        for j in range(2):
            for mi in range(3):
                st_copy(j, mi).start()
        cp_m = pltpu.make_async_copy(mem0_hbm, mem0_ref, sem_x.at[2])
        cp_m.start()

        def prenorm(r):
            x = x_v[r, :].astype(F32)
            xs_ref[r, :] = x
            ln_ref[r, :] = _ln(x)

        cp_x0.wait()
        prenorm(pl.ds(0, X0))
        h_ref[pl.ds(0, HALO), :] = jnp.zeros((HALO, D), F32)
        h_ref[pl.ds(HALO + S, HALO), :] = jnp.zeros((HALO, D), F32)

        def relayout(j):
            r0 = pl.multiple_of(j * PW, 128)
            for mi, dst in enumerate((wq_s, wk_s, wv_s)):
                a = stage[mi, pl.ds(r0, 128), :]
                b = stage[mi, pl.ds(r0 + Dh, 128), :]
                t = jnp.concatenate([stage[mi, pl.ds(r0 + 128, 64), :],
                                     stage[mi, pl.ds(r0 + Dh + 128, 64), :]], axis=0)
                for n, v in enumerate((a, b, t)):
                    dst[3 * j + n] = pltpu.bitcast(v.T, I32)

        def pair_w(w_s, j):
            return jnp.concatenate(
                [pltpu.bitcast(w_s[3 * j + t], BF16) for t in range(3)], axis=1)

        def lead_proj(j):
            rows = ln_ref[pl.ds(0, LEAD), :]
            for mi, w_s in enumerate((wq_s, wk_s, wv_s)):
                ring[mi, j, pl.ds(0, LEAD), :] = _dot(rows, pair_w(w_s, j))

        def arrive(j):
            for mi in range(3):
                st_copy(j, mi).wait()

            @pl.when(j + AHEAD < NP)
            def _():
                for mi in range(3):
                    st_copy(j + AHEAD, mi).start()

            @pl.when(j + AHEAD == NP)
            def _():
                cp_x1.start()
                w_cps[0].start()

        for j in range(2, RAMP + 1):
            for mi in range(3):
                st_copy(j - 2, mi).wait()
                st_copy(2 * j - 2, mi).start()
                st_copy(2 * j - 1, mi).start()
            relayout(j - 2)
            if j > 2:
                lead_proj(j - 3)

        def startup(j, _):
            arrive(j)
            lead_proj(j - 1)
            relayout(j)
            return 0
        with jax.named_scope('startup'):
            jax.lax.fori_loop(RAMP - 1, NP, startup, 0)
            lead_proj(NP - 1)
        cp_x1.wait()
        cp_m.wait()

        def init_tile(t, _):
            prenorm(pl.ds(pl.multiple_of(X0 + t * IT, 8), IT))
            return 0
        jax.lax.fori_loop(0, (S - X0) // IT, init_tile, 0)
        with jax.named_scope('wait_wo'):
            w_cps[0].wait()
        for cp in w_cps[1:]:
            cp.start()

        def a_step(lead, s, mem):
            r = pl.ds(pl.multiple_of(s * SEG, SEG), SEG)
            if lead:
                p0 = LEAD + s * XR
                hrows = jnp.concatenate([mem, ln_ref[pl.ds(pl.multiple_of(p0, 8), XR), :]], axis=0)
                wpos = pl.ds(pl.multiple_of(jax.lax.rem(p0, RING), 8), XR)
                rpos = pl.ds(pl.multiple_of(jax.lax.rem(s * SEG, RING), 8), SEG)
            else:
                hrows = jnp.concatenate([mem, ln_ref[r, :]], axis=0)
            lo64 = jax.lax.broadcasted_iota(I32, (L, 128), 1) < 64
            zero = jnp.zeros((L, 128), F32)
            rowb = jax.lax.broadcasted_iota(I32, (PP * L, 2 * L), 0) % L
            colb = jax.lax.broadcasted_iota(I32, (PP * L, 2 * L), 1)
            lob = colb < L
            maskb = (rowb < M) | (rowb >= jnp.where(lob, colb, colb - L))

            def proj(mi, g):
                w_s = (wq_s, wk_s, wv_s)[mi]
                y = _dot(hrows, jnp.concatenate(
                    [pair_w(w_s, g * PP + u) for u in range(PP)], axis=1))
                if lead:
                    for u in range(PP):
                        ring[mi, g * PP + u, wpos, :] = y[M:, u * PW:(u + 1) * PW]
                    y = jnp.concatenate([y[:M, :], jnp.concatenate(
                        [ring[mi, g * PP + u, rpos, :] for u in range(PP)], axis=1)], axis=0)
                return y

            def stack(x, j):
                t0 = x[:, 384 * j:384 * j + 128]
                t1 = x[:, 384 * j + 128:384 * j + 256]
                t2 = x[:, 384 * j + 256:384 * j + 384]
                top = jnp.concatenate([t0, zero, jnp.where(lo64, t2, 0.0)], axis=1)
                bot = jnp.concatenate([zero, t1, jnp.where(lo64, 0.0, t2)], axis=1)
                return jnp.concatenate([top, bot], axis=0).astype(BF16)

            def scores(q, k):
                return jnp.concatenate(
                    [_dot_nt(q[:, 384 * j:384 * (j + 1)], stack(k, j)) for j in range(PP)],
                    axis=0) * scale

            def softmax(sc):
                sc = jnp.where(maskb, sc, _NEG)
                m_lo = jnp.max(jnp.where(lob, sc, -jnp.inf), axis=1, keepdims=True)
                m_hi = jnp.max(jnp.where(lob, -jnp.inf, sc), axis=1, keepdims=True)
                e = jnp.exp(sc - jnp.where(lob, m_lo, m_hi))
                s_lo = jnp.sum(jnp.where(lob, e, 0.0), axis=1, keepdims=True)
                s_hi = jnp.sum(jnp.where(lob, 0.0, e), axis=1, keepdims=True)
                return e / jnp.where(lob, s_lo, s_hi)

            def pv(p, v):
                return jnp.concatenate(
                    [_dot(p[j * L:(j + 1) * L], stack(v, j)) for j in range(PP)], axis=1)

            def out_proj(g, o):
                rows = []
                for j in range(PP):
                    r0 = (g * PP + j) * 2 * Dh
                    rows += [wo_ref[r0:r0 + 128, :], wo_ref[r0 + Dh:r0 + Dh + 128, :],
                             wo_ref[r0 + 128:r0 + Dh, :], wo_ref[r0 + Dh + 128:r0 + 2 * Dh, :]]
                return _dot(o, jnp.concatenate(rows, axis=0))

            qkv = [None] * G
            sc = [None] * G
            p = [None] * G
            o = [None] * G
            acc = None
            for it in range(G + WO_LAG):
                if it < G:
                    qkv[it] = (proj(0, it), proj(1, it), proj(2, it))
                if 0 <= it - 1 < G:
                    sc[it - 1] = scores(qkv[it - 1][0], qkv[it - 1][1])
                if 0 <= it - 2 < G:
                    o[it - 2] = pv(p[it - 2], qkv[it - 2][2])
                if 0 <= it - 1 < G:
                    p[it - 1] = softmax(sc[it - 1])
                if 0 <= it - WO_LAG < G:
                    t = out_proj(it - WO_LAG, o[it - WO_LAG])
                    acc = t if acc is None else acc + t
            xs_ref[r, :] = xs_ref[r, :] + acc[M:, :]
            return acc[:M, :]

        def b1_in(t):
            return xs_ref[pl.ds(pl.multiple_of(t * RT, RT), RT), :]

        def b1_mid(t, x):
            xl = _ln(x)
            xl_ref[pl.ds(pl.multiple_of(t * RT, RT), RT), :] = xl
            return _dot(_ln(xl).astype(BF16), w1_ref[...])

        def b1_out(t, h1):
            h_ref[pl.ds(pl.multiple_of(t * RT, RT) + HALO, RT), :] = _gelu(h1)

        def b2_in(t):
            r0 = pl.multiple_of(t * RT, RT)
            pieces = []
            shifts = (-1, 1, -2, 2)
            for lt in range(D // 128):
                c0 = lt * 128
                win = h_ref[pl.ds(r0, RT + 2 * HALO), pl.ds(c0, 128)]
                g_lo, g_hi = c0 // c, min((c0 + 127) // c, 3)
                a = win[HALO + shifts[g_lo]: HALO + shifts[g_lo] + RT]
                if g_hi != g_lo:
                    bb = win[HALO + shifts[g_hi]: HALO + shifts[g_hi] + RT]
                    lane = jax.lax.broadcasted_iota(I32, (RT, 128), 1) + c0
                    a = jnp.where(lane < g_hi * c, a, bb)
                pieces.append(a)
            hs_in = jnp.concatenate(pieces, axis=1).astype(BF16)
            return hs_in, xl_ref[pl.ds(r0, RT), :], xs_ref[pl.ds(r0, RT), :]

        def b_tile(t, ahead, last):
            r = pl.ds(pl.multiple_of(t * RT, RT), RT)
            hs_in, xl_t, x_t = b2_in(t)
            if ahead:
                x_n = b1_in(t + 2)
            x1 = xl_t + _dot(hs_in, w2_ref[...])
            if ahead:
                h1 = b1_mid(t + 2, x_n)
            g = _gelu(_dot(_ln(x1).astype(BF16), w3_ref[...]))
            if ahead:
                b1_out(t + 2, h1)
            xn = x_t + (x1 + _dot(g.astype(BF16), w4_ref[...]))
            if last:
                x_v[r, :] = xn.astype(BF16)
                out_copy(t).start()
            else:
                xs_ref[r, :] = xn
                ln_ref[r, :] = _ln(xn)

        def out_copy(t):
            r = pl.ds(pl.multiple_of(t * RT, RT), RT)
            return pltpu.make_async_copy(x_v.at[r], out_hbm.at[r], sem_o.at[t])

        def b1_tile(t, _):
            b1_out(t, b1_mid(t, b1_in(t)))
            return 0

        for layer in range(2):
            last = layer == 1
            with jax.named_scope('A%d' % layer):
                mem = mem0_ref[...].astype(F32)
                if layer == 0:
                    mem = jax.lax.fori_loop(0, NLEAD, functools.partial(a_step, True), mem, unroll=UNR)
                jax.lax.fori_loop(NLEAD if layer == 0 else 0, NSEG,
                                  functools.partial(a_step, False), mem, unroll=UNR)
            if layer == 0:
                for cp in w_cps[1:]:
                    cp.wait()
            with jax.named_scope('Bp1_%d' % layer):
                jax.lax.fori_loop(0, 2, b1_tile, 0)
            with jax.named_scope('Bp2_%d' % layer):
                jax.lax.fori_loop(0, NT - 2, functools.partial(_b_body, b_tile, True, last), 0)
            with jax.named_scope('Bp3_%d' % layer):
                jax.lax.fori_loop(NT - 2, NT, functools.partial(_b_body, b_tile, False, last), 0)
        for t in range(NT):
            out_copy(t).wait()

    return kernel


def _b_body(fn, ahead, last, t, carry):
    fn(t, ahead, last)
    return carry


@functools.partial(jax.jit, static_argnames=("A_seg_len",))
def pallas_interleave_layers__memory_aug_recurrent_mem_tr__mixer_s_mlp__prompt_kernel(
    A_x: jax.Array,
    A_mem0: jax.Array,
    A_Wq: jax.Array,
    A_Wk: jax.Array,
    A_Wv: jax.Array,
    A_Wo: jax.Array,
    A_seg_len,
    B_x: jax.Array,
    B_w1: jax.Array,
    B_w2: jax.Array,
    B_w3: jax.Array,
    B_w4: jax.Array,
):
    del B_x
    B, S, D = A_x.shape
    assert B == 1
    H, Dh = A_Wq.shape[1], A_Wq.shape[2]
    M = A_mem0.shape[1]
    SEG = int(A_seg_len)
    F = B_w3.shape[1]
    kernel = _make_kernel(S, D, H, Dh, M, SEG, F)
    hbm = pl.BlockSpec(memory_space=pl.ANY)
    nt = 3 * H // 2

    def wt(w):
        return jnp.transpose(w, (1, 2, 0)).reshape(H * Dh, D)

    out = pl.pallas_call(
        kernel,
        out_shape=jax.ShapeDtypeStruct((S, D), A_x.dtype),
        in_specs=[hbm] * 10,
        out_specs=hbm,
        scratch_shapes=[
            pltpu.VMEM((S, D), BF16),
            pltpu.VMEM((3, H * Dh, D), BF16),
            pltpu.VMEM((nt, D // 2, 128), I32),
            pltpu.VMEM((nt, D // 2, 128), I32),
            pltpu.VMEM((nt, D // 2, 128), I32),
            pltpu.VMEM((H * Dh, D), BF16),
            pltpu.VMEM((D, D), BF16),
            pltpu.VMEM((D, D), BF16),
            pltpu.VMEM((D, F), BF16),
            pltpu.VMEM((F, D), BF16),
            pltpu.VMEM((S, D), F32),
            pltpu.VMEM((S, D), F32),
            pltpu.VMEM((S, D), F32),
            pltpu.VMEM((S + 16, D), F32),
            pltpu.VMEM((3, 16, 384, 384), F32),
            pltpu.VMEM((M, D), BF16),
            pltpu.SemaphoreType.DMA((3,)),
            pltpu.SemaphoreType.DMA((48,)),
            pltpu.SemaphoreType.DMA((5,)),
            pltpu.SemaphoreType.DMA((8,)),
        ],
        compiler_params=pltpu.CompilerParams(vmem_limit_bytes=120 * 1024 * 1024),
    )(
        A_mem0.reshape(M, D), A_x.reshape(S, D), wt(A_Wq), wt(A_Wk), wt(A_Wv),
        A_Wo.reshape(H * Dh, D), B_w1, B_w2, B_w3, B_w4,
    )
    return out.reshape(B, S, D)
```

```python
import functools

import jax
import jax.numpy as jnp
import numpy as np
import jax.experimental.pallas as pl
import jax.experimental.pallas.tpu as pltpu

F32 = jnp.float32
BF16 = jnp.bfloat16
I32 = jnp.int32
_NEG = -1000000000.0


def _ln(x, eps=1e-05):
    m = jnp.mean(x, axis=-1, keepdims=True)
    d = x - m
    v = jnp.mean(d * d, axis=-1, keepdims=True)
    return d * jax.lax.rsqrt(v + eps)


def _gelu(x):
    c = float(np.sqrt(2.0 / np.pi))
    return 0.5 * x * (1.0 + jnp.tanh(c * (x + 0.044715 * (x * x * x))))


def _dot(a, b):
    return jnp.dot(a, b, preferred_element_type=F32)


def _dot_nt(a, b):
    return jax.lax.dot_general(a, b, (((1,), (1,)), ((), ())), preferred_element_type=F32)


def _make_kernel(S, D, H, Dh, M, SEG, F, G=8, WO_LAG=4, RAMP=4, UNR=2):
    L = M + SEG
    NSEG = S // SEG
    NP = H // 2
    PP = NP // G
    scale = Dh ** (-0.5)
    RT = 256
    NT = S // RT
    HALO = 8
    c = D // 4
    PW = 2 * Dh
    AHEAD = RAMP + 1
    XR = 24
    LEAD = 12 * XR
    NLEAD = LEAD // (SEG - XR)
    RING = 384
    X0 = LEAD + XR
    XW = 8
    X1 = X0 + XW * XR + 8
    assert Dh == 192 and D % 128 == 0
    assert RING % XR == 0 and RING % SEG == 0 and RING >= LEAD + XR

    def kernel(mem0_hbm, x_hbm, wq_hbm, wk_hbm, wv_hbm, wo_hbm,
               w1_hbm, w2_hbm, w3_hbm, w4_hbm, out_hbm,
               x_v, stage, wq_s, wk_s, wv_s, wo_ref, w1_ref, w2_ref, w3_ref, w4_ref,
               xs_ref, ln_ref, xl_ref, h_ref, ring, mem0_ref, sem_x, sem_st, sem_w, sem_o):
        def st_copy(j, mi):
            rows = pl.ds(pl.multiple_of(j * PW, 128), PW)
            return pltpu.make_async_copy(
                (wq_hbm, wk_hbm, wv_hbm)[mi].at[rows], stage.at[mi, rows], sem_st.at[3 * j + mi])

        cp_x0 = pltpu.make_async_copy(x_hbm.at[pl.ds(0, X1)], x_v.at[pl.ds(0, X1)], sem_x.at[0])
        cp_x1 = pltpu.make_async_copy(
            x_hbm.at[pl.ds(X1, S - X1)], x_v.at[pl.ds(X1, S - X1)], sem_x.at[1])
        w_cps = [pltpu.make_async_copy(src, dst, sem_w.at[wi])
                 for wi, (src, dst) in enumerate(
                     ((wo_hbm, wo_ref), (w1_hbm, w1_ref), (w2_hbm, w2_ref),
                      (w3_hbm, w3_ref), (w4_hbm, w4_ref)))]
        cp_x0.start()
        for j in range(2):
            for mi in range(3):
                st_copy(j, mi).start()
        cp_m = pltpu.make_async_copy(mem0_hbm, mem0_ref, sem_x.at[2])
        cp_m.start()

        def prenorm(r):
            x = x_v[r, :].astype(F32)
            xs_ref[r, :] = x
            ln_ref[r, :] = _ln(x)

        cp_x0.wait()
        prenorm(pl.ds(0, X0))
        h_ref[pl.ds(0, HALO), :] = jnp.zeros((HALO, D), F32)
        h_ref[pl.ds(HALO + S, HALO), :] = jnp.zeros((HALO, D), F32)

        def relayout(j):
            r0 = pl.multiple_of(j * PW, 128)
            for mi, dst in enumerate((wq_s, wk_s, wv_s)):
                a = stage[mi, pl.ds(r0, 128), :]
                b = stage[mi, pl.ds(r0 + Dh, 128), :]
                t = jnp.concatenate([stage[mi, pl.ds(r0 + 128, 64), :],
                                     stage[mi, pl.ds(r0 + Dh + 128, 64), :]], axis=0)
                for n, v in enumerate((a, b, t)):
                    dst[3 * j + n] = pltpu.bitcast(v.T, I32)

        def pair_w(w_s, j):
            return jnp.concatenate(
                [pltpu.bitcast(w_s[3 * j + t], BF16) for t in range(3)], axis=1)

        def lead_proj(j):
            rows = ln_ref[pl.ds(0, LEAD), :]
            for mi, w_s in enumerate((wq_s, wk_s, wv_s)):
                ring[mi, j, pl.ds(0, LEAD), :] = _dot(rows, pair_w(w_s, j))

        def arrive(j):
            for mi in range(3):
                st_copy(j, mi).wait()

            @pl.when(j + AHEAD < NP)
            def _():
                for mi in range(3):
                    st_copy(j + AHEAD, mi).start()

            @pl.when(j + AHEAD == NP)
            def _():
                w_cps[0].start()

        for j in range(2, RAMP + 1):
            for mi in range(3):
                st_copy(j - 2, mi).wait()
                st_copy(2 * j - 2, mi).start()
                st_copy(2 * j - 1, mi).start()
            relayout(j - 2)
            if j > 2:
                lead_proj(j - 3)

        def startup(j, _):
            arrive(j)
            lead_proj(j - 1)
            relayout(j)
            return 0
        with jax.named_scope('startup'):
            jax.lax.fori_loop(RAMP - 1, NP, startup, 0)
            lead_proj(NP - 1)
        cp_m.wait()
        w_cps[0].wait()
        cp_x1.start()
        for cp in w_cps[1:]:
            cp.start()

        def a_step(layer, lead, s, mem):
            r = pl.ds(pl.multiple_of(s * SEG, SEG), SEG)
            n0 = X0 + s * XR if lead else (s + 1) * SEG
            n_src = pl.ds(pl.multiple_of(jnp.minimum(n0, S - SEG), 8), SEG)
            n_dst = pl.ds(pl.multiple_of(n0, 8), SEG)
            if layer == 0:
                x_next = x_v[n_src, :].astype(F32)
            else:
                x_next = xs_ref[n_src, :]
            if lead:
                p0 = LEAD + s * XR
                hrows = jnp.concatenate([mem, ln_ref[pl.ds(pl.multiple_of(p0, 8), XR), :]], axis=0)
                wpos = pl.ds(pl.multiple_of(jax.lax.rem(p0, RING), 8), XR)
                rpos = pl.ds(pl.multiple_of(jax.lax.rem(s * SEG, RING), 8), SEG)
            else:
                hrows = jnp.concatenate([mem, ln_ref[r, :]], axis=0)
            lo64 = jax.lax.broadcasted_iota(I32, (L, 128), 1) < 64
            zero = jnp.zeros((L, 128), F32)
            rowb = jax.lax.broadcasted_iota(I32, (PP * L, 2 * L), 0) % L
            colb = jax.lax.broadcasted_iota(I32, (PP * L, 2 * L), 1)
            lob = colb < L
            maskb = (rowb < M) | (rowb >= jnp.where(lob, colb, colb - L))

            def proj(mi, g):
                w_s = (wq_s, wk_s, wv_s)[mi]
                y = _dot(hrows, jnp.concatenate(
                    [pair_w(w_s, g * PP + u) for u in range(PP)], axis=1))
                if lead:
                    for u in range(PP):
                        ring[mi, g * PP + u, wpos, :] = y[M:, u * PW:(u + 1) * PW]
                    y = jnp.concatenate([y[:M, :], jnp.concatenate(
                        [ring[mi, g * PP + u, rpos, :] for u in range(PP)], axis=1)], axis=0)
                return y

            def stack(x, j):
                t0 = x[:, 384 * j:384 * j + 128]
                t1 = x[:, 384 * j + 128:384 * j + 256]
                t2 = x[:, 384 * j + 256:384 * j + 384]
                top = jnp.concatenate([t0, zero, jnp.where(lo64, t2, 0.0)], axis=1)
                bot = jnp.concatenate([zero, t1, jnp.where(lo64, 0.0, t2)], axis=1)
                return jnp.concatenate([top, bot], axis=0).astype(BF16)

            def scores(q, k):
                return jnp.concatenate(
                    [_dot_nt(q[:, 384 * j:384 * (j + 1)], stack(k, j)) for j in range(PP)],
                    axis=0) * scale

            def softmax(sc):
                sc = jnp.where(maskb, sc, _NEG)
                m_lo = jnp.max(jnp.where(lob, sc, -jnp.inf), axis=1, keepdims=True)
                m_hi = jnp.max(jnp.where(lob, -jnp.inf, sc), axis=1, keepdims=True)
                e = jnp.exp(sc - jnp.where(lob, m_lo, m_hi))
                s_lo = jnp.sum(jnp.where(lob, e, 0.0), axis=1, keepdims=True)
                s_hi = jnp.sum(jnp.where(lob, 0.0, e), axis=1, keepdims=True)
                return e / jnp.where(lob, s_lo, s_hi)

            def pv(p, v):
                return jnp.concatenate(
                    [_dot(p[j * L:(j + 1) * L], stack(v, j)) for j in range(PP)], axis=1)

            def out_proj(g, o):
                rows = []
                for j in range(PP):
                    r0 = (g * PP + j) * 2 * Dh
                    rows += [wo_ref[r0:r0 + 128, :], wo_ref[r0 + Dh:r0 + Dh + 128, :],
                             wo_ref[r0 + 128:r0 + Dh, :], wo_ref[r0 + Dh + 128:r0 + 2 * Dh, :]]
                return _dot(o, jnp.concatenate(rows, axis=0))

            qkv = [None] * G
            sc = [None] * G
            p = [None] * G
            o = [None] * G
            acc = None
            for it in range(G + WO_LAG):
                if it < G:
                    qkv[it] = (proj(0, it), proj(1, it), proj(2, it))
                if 0 <= it - 1 < G:
                    sc[it - 1] = scores(qkv[it - 1][0], qkv[it - 1][1])
                if 0 <= it - 2 < G:
                    o[it - 2] = pv(p[it - 2], qkv[it - 2][2])
                if 0 <= it - 1 < G:
                    p[it - 1] = softmax(sc[it - 1])
                if 0 <= it - WO_LAG < G:
                    t = out_proj(it - WO_LAG, o[it - WO_LAG])
                    acc = t if acc is None else acc + t
            xs_ref[r, :] = xs_ref[r, :] + acc[M:, :]
            if layer == 0:
                xs_ref[n_dst, :] = x_next
            ln_ref[n_dst, :] = _ln(x_next)
            return acc[:M, :]

        def lead_steps(i, mem):
            @pl.when(i == XW // UNR)
            def _():
                cp_x1.wait()
            for u in range(UNR):
                mem = a_step(0, True, i * UNR + u, mem)
            return mem

        def b1_in(t):
            return xs_ref[pl.ds(pl.multiple_of(t * RT, RT), RT), :]

        def b1_mid(t, x):
            xl = _ln(x)
            xl_ref[pl.ds(pl.multiple_of(t * RT, RT), RT), :] = xl
            return _dot(_ln(xl).astype(BF16), w1_ref[...])

        def b1_out(t, h1):
            h_ref[pl.ds(pl.multiple_of(t * RT, RT) + HALO, RT), :] = _gelu(h1)

        def b2_in(t):
            r0 = pl.multiple_of(t * RT, RT)
            pieces = []
            shifts = (-1, 1, -2, 2)
            for lt in range(D // 128):
                c0 = lt * 128
                win = h_ref[pl.ds(r0, RT + 2 * HALO), pl.ds(c0, 128)]
                g_lo, g_hi = c0 // c, min((c0 + 127) // c, 3)
                a = win[HALO + shifts[g_lo]: HALO + shifts[g_lo] + RT]
                if g_hi != g_lo:
                    bb = win[HALO + shifts[g_hi]: HALO + shifts[g_hi] + RT]
                    lane = jax.lax.broadcasted_iota(I32, (RT, 128), 1) + c0
                    a = jnp.where(lane < g_hi * c, a, bb)
                pieces.append(a)
            hs_in = jnp.concatenate(pieces, axis=1).astype(BF16)
            return hs_in, xl_ref[pl.ds(r0, RT), :], xs_ref[pl.ds(r0, RT), :]

        def b_tile(t, ahead, last):
            r = pl.ds(pl.multiple_of(t * RT, RT), RT)
            hs_in, xl_t, x_t = b2_in(t)
            if ahead:
                x_n = b1_in(t + 2)
            x1 = xl_t + _dot(hs_in, w2_ref[...])
            if ahead:
                h1 = b1_mid(t + 2, x_n)
            g = _gelu(_dot(_ln(x1).astype(BF16), w3_ref[...]))
            if ahead:
                b1_out(t + 2, h1)
            xn = x_t + (x1 + _dot(g.astype(BF16), w4_ref[...]))
            if last:
                x_v[r, :] = xn.astype(BF16)
                out_copy(t).start()
            else:
                xs_ref[r, :] = xn

        def out_copy(t):
            r = pl.ds(pl.multiple_of(t * RT, RT), RT)
            return pltpu.make_async_copy(x_v.at[r], out_hbm.at[r], sem_o.at[t])

        def b1_tile(t, _):
            b1_out(t, b1_mid(t, b1_in(t)))
            return 0

        for layer in range(2):
            last = layer == 1
            with jax.named_scope('A%d' % layer):
                mem = mem0_ref[...].astype(F32)
                if layer == 0:
                    mem = jax.lax.fori_loop(0, NLEAD // UNR, lead_steps, mem)
                jax.lax.fori_loop(NLEAD if layer == 0 else 0, NSEG,
                                  functools.partial(a_step, layer, False), mem, unroll=UNR)
            if layer == 0:
                for cp in w_cps[1:]:
                    cp.wait()
            with jax.named_scope('Bp1_%d' % layer):
                jax.lax.fori_loop(0, 2, b1_tile, 0)
            with jax.named_scope('Bp2_%d' % layer):
                jax.lax.fori_loop(0, NT - 2, functools.partial(_b_body, b_tile, True, last), 0)
            with jax.named_scope('Bp3_%d' % layer):
                jax.lax.fori_loop(NT - 2, NT, functools.partial(_b_body, b_tile, False, last), 0)
            if not last:
                ln_ref[pl.ds(0, SEG), :] = _ln(xs_ref[pl.ds(0, SEG), :])
        for t in range(NT):
            out_copy(t).wait()

    return kernel


def _b_body(fn, ahead, last, t, carry):
    fn(t, ahead, last)
    return carry


@functools.partial(jax.jit, static_argnames=("A_seg_len",))
def pallas_interleave_layers__memory_aug_recurrent_mem_tr__mixer_s_mlp__prompt_kernel(
    A_x: jax.Array,
    A_mem0: jax.Array,
    A_Wq: jax.Array,
    A_Wk: jax.Array,
    A_Wv: jax.Array,
    A_Wo: jax.Array,
    A_seg_len,
    B_x: jax.Array,
    B_w1: jax.Array,
    B_w2: jax.Array,
    B_w3: jax.Array,
    B_w4: jax.Array,
):
    del B_x
    B, S, D = A_x.shape
    assert B == 1
    H, Dh = A_Wq.shape[1], A_Wq.shape[2]
    M = A_mem0.shape[1]
    SEG = int(A_seg_len)
    F = B_w3.shape[1]
    kernel = _make_kernel(S, D, H, Dh, M, SEG, F)
    hbm = pl.BlockSpec(memory_space=pl.ANY)
    nt = 3 * H // 2

    def wt(w):
        return jnp.transpose(w, (1, 2, 0)).reshape(H * Dh, D)

    out = pl.pallas_call(
        kernel,
        out_shape=jax.ShapeDtypeStruct((S, D), A_x.dtype),
        in_specs=[hbm] * 10,
        out_specs=hbm,
        scratch_shapes=[
            pltpu.VMEM((S, D), BF16),
            pltpu.VMEM((3, H * Dh, D), BF16),
            pltpu.VMEM((nt, D // 2, 128), I32),
            pltpu.VMEM((nt, D // 2, 128), I32),
            pltpu.VMEM((nt, D // 2, 128), I32),
            pltpu.VMEM((H * Dh, D), BF16),
            pltpu.VMEM((D, D), BF16),
            pltpu.VMEM((D, D), BF16),
            pltpu.VMEM((D, F), BF16),
            pltpu.VMEM((F, D), BF16),
            pltpu.VMEM((S + SEG, D), F32),
            pltpu.VMEM((S + SEG, D), F32),
            pltpu.VMEM((S, D), F32),
            pltpu.VMEM((S + 16, D), F32),
            pltpu.VMEM((3, 16, 384, 384), F32),
            pltpu.VMEM((M, D), BF16),
            pltpu.SemaphoreType.DMA((3,)),
            pltpu.SemaphoreType.DMA((48,)),
            pltpu.SemaphoreType.DMA((5,)),
            pltpu.SemaphoreType.DMA((8,)),
        ],
        compiler_params=pltpu.CompilerParams(vmem_limit_bytes=120 * 1024 * 1024),
    )(
        A_mem0.reshape(M, D), A_x.reshape(S, D), wt(A_Wq), wt(A_Wk), wt(A_Wv),
        A_Wo.reshape(H * Dh, D), B_w1, B_w2, B_w3, B_w4,
    )
    return out.reshape(B, S, D)
```

```python
import functools

import jax
import jax.numpy as jnp
import numpy as np
import jax.experimental.pallas as pl
import jax.experimental.pallas.tpu as pltpu

F32 = jnp.float32
BF16 = jnp.bfloat16
I32 = jnp.int32
_NEG = -1000000000.0


def _ln(x, eps=1e-05):
    m = jnp.mean(x, axis=-1, keepdims=True)
    d = x - m
    v = jnp.mean(d * d, axis=-1, keepdims=True)
    return d * jax.lax.rsqrt(v + eps)


def _gelu(x):
    c = float(np.sqrt(2.0 / np.pi))
    return 0.5 * x * (1.0 + jnp.tanh(c * (x + 0.044715 * (x * x * x))))


def _dot(a, b):
    return jnp.dot(a, b, preferred_element_type=F32)


def _dot_nt(a, b):
    return jax.lax.dot_general(a, b, (((1,), (1,)), ((), ())), preferred_element_type=F32)


def _make_kernel(S, D, H, Dh, M, SEG, F, G=8, WO_LAG=4, RAMP=4, UNR=2, BU=2, MD=2):
    L = M + SEG
    NSEG = S // SEG
    NP = H // 2
    PP = NP // G
    scale = Dh ** (-0.5)
    RT = 128
    NT = S // RT
    HALO = 8
    c = D // 4
    PW = 2 * Dh
    AHEAD = RAMP + 1
    XR = 24
    LEAD = 12 * XR
    NLEAD = LEAD // (SEG - XR)
    RING = 384
    X0 = LEAD + XR
    XW = 8
    X1 = X0 + XW * XR + 8
    assert Dh == 192 and D % 128 == 0
    assert RING % XR == 0 and RING % SEG == 0 and RING >= LEAD + XR

    def kernel(mem0_hbm, x_hbm, wq_hbm, wk_hbm, wv_hbm, wo_hbm,
               w1_hbm, w2_hbm, w3_hbm, w4_hbm, out_hbm,
               x_v, stage, wq_s, wk_s, wv_s, wo_ref, w1_ref, w2_ref, w3_ref, w4_ref,
               xs_ref, ln_ref, xl_ref, h_ref, ring, mem0_ref, sem_x, sem_st, sem_w, sem_o):
        def st_copy(j, mi):
            rows = pl.ds(pl.multiple_of(j * PW, 128), PW)
            return pltpu.make_async_copy(
                (wq_hbm, wk_hbm, wv_hbm)[mi].at[rows], stage.at[mi, rows], sem_st.at[3 * j + mi])

        cp_x0 = pltpu.make_async_copy(x_hbm.at[pl.ds(0, X1)], x_v.at[pl.ds(0, X1)], sem_x.at[0])
        cp_x1 = pltpu.make_async_copy(
            x_hbm.at[pl.ds(X1, S - X1)], x_v.at[pl.ds(X1, S - X1)], sem_x.at[1])
        w_cps = [pltpu.make_async_copy(src, dst, sem_w.at[wi])
                 for wi, (src, dst) in enumerate(
                     ((wo_hbm, wo_ref), (w1_hbm, w1_ref), (w2_hbm, w2_ref),
                      (w3_hbm, w3_ref), (w4_hbm, w4_ref)))]
        cp_x0.start()
        for j in range(2):
            for mi in range(3):
                st_copy(j, mi).start()
        cp_m = pltpu.make_async_copy(mem0_hbm, mem0_ref, sem_x.at[2])
        cp_m.start()

        def prenorm(r):
            x = x_v[r, :].astype(F32)
            xs_ref[r, :] = x
            ln_ref[r, :] = _ln(x)

        cp_x0.wait()
        prenorm(pl.ds(0, X0))
        h_ref[pl.ds(0, HALO), :] = jnp.zeros((HALO, D), F32)

        def relayout(j):
            r0 = pl.multiple_of(j * PW, 128)
            for mi, dst in enumerate((wq_s, wk_s, wv_s)):
                a = stage[mi, pl.ds(r0, 128), :]
                b = stage[mi, pl.ds(r0 + Dh, 128), :]
                t = jnp.concatenate([stage[mi, pl.ds(r0 + 128, 64), :],
                                     stage[mi, pl.ds(r0 + Dh + 128, 64), :]], axis=0)
                for n, v in enumerate((a, b, t)):
                    dst[3 * j + n] = pltpu.bitcast(v.T, I32)

        def pair_w(w_s, j):
            return jnp.concatenate(
                [pltpu.bitcast(w_s[3 * j + t], BF16) for t in range(3)], axis=1)

        def lead_proj(j):
            rows = ln_ref[pl.ds(0, LEAD), :]
            for mi, w_s in enumerate((wq_s, wk_s, wv_s)):
                ring[mi, j // PP, pl.ds(0, LEAD), pl.ds(pl.multiple_of((j % PP) * PW, 128), PW)] = _dot(rows, pair_w(w_s, j))

        def arrive(j):
            for mi in range(3):
                st_copy(j, mi).wait()

            @pl.when(j + AHEAD < NP)
            def _():
                for mi in range(3):
                    st_copy(j + AHEAD, mi).start()

            @pl.when(j + AHEAD == NP)
            def _():
                w_cps[0].start()
                w_cps[1].start()

        for j in range(2, RAMP + 1):
            for mi in range(3):
                st_copy(j - 2, mi).wait()
                st_copy(2 * j - 2, mi).start()
                st_copy(2 * j - 1, mi).start()
            relayout(j - 2)
            if j > 2:
                lead_proj(j - 3)

        def startup(j, _):
            arrive(j)
            lead_proj(j - 1)
            relayout(j)
            return 0
        with jax.named_scope('startup'):
            jax.lax.fori_loop(RAMP - 1, NP, startup, 0)
            lead_proj(NP - 1)
        cp_m.wait()
        w_cps[0].wait()
        w_cps[1].wait()
        cp_x1.start()
        for cp in w_cps[2:]:
            cp.start()

        def mixer1(x, dst, n):
            xl = _ln(x)
            xl_ref[pl.ds(pl.multiple_of(dst, 8), n), :] = xl
            h_ref[pl.ds(pl.multiple_of(dst + HALO, 8), n), :] = _gelu(
                _dot(_ln(xl).astype(BF16), w1_ref[...]))

        def a_step(layer, lead, s, mem):
            r = pl.ds(pl.multiple_of(s * SEG, SEG), SEG)
            m_src = pl.ds(pl.multiple_of(jnp.maximum(s - MD, 0) * SEG, SEG), SEG)
            x_mix = xs_ref[m_src, :]
            n0 = X0 + s * XR if lead else (s + 1) * SEG
            n_src = pl.ds(pl.multiple_of(jnp.minimum(n0, S - SEG), 8), SEG)
            n_dst = pl.ds(pl.multiple_of(n0, 8), SEG)
            if layer == 0:
                x_next = x_v[n_src, :].astype(F32)
            else:
                x_next = xs_ref[n_src, :]
            if lead:
                p0 = LEAD + s * XR
                hrows = jnp.concatenate(
                    [mem, ln_ref[pl.ds(pl.multiple_of(p0, 8), XR), :]], axis=0).astype(BF16)
                wpos = pl.ds(pl.multiple_of(jax.lax.rem(p0, RING), 8), XR)
                rpos = pl.ds(pl.multiple_of(jax.lax.rem(s * SEG, RING), 8), SEG)
            else:
                hrows = jnp.concatenate([mem, ln_ref[r, :]], axis=0)
            lo64 = jax.lax.broadcasted_iota(I32, (L, 128), 1) < 64
            zero = jnp.zeros((L, 128), F32)
            rowb = jax.lax.broadcasted_iota(I32, (PP * L, 2 * L), 0) % L
            colb = jax.lax.broadcasted_iota(I32, (PP * L, 2 * L), 1)
            lob = colb < L
            maskb = (rowb < M) | (rowb >= jnp.where(lob, colb, colb - L))

            def proj(mi, g):
                w_s = (wq_s, wk_s, wv_s)[mi]
                y = _dot(hrows, jnp.concatenate(
                    [pair_w(w_s, g * PP + u) for u in range(PP)], axis=1))
                if lead:
                    ring[mi, g, wpos, :] = y[M:, :]
                    y = jnp.concatenate([y[:M, :], ring[mi, g, rpos, :]], axis=0)
                return y

            def stack(x, j):
                t0 = x[:, 384 * j:384 * j + 128]
                t1 = x[:, 384 * j + 128:384 * j + 256]
                t2 = x[:, 384 * j + 256:384 * j + 384]
                top = jnp.concatenate([t0, zero, jnp.where(lo64, t2, 0.0)], axis=1)
                bot = jnp.concatenate([zero, t1, jnp.where(lo64, 0.0, t2)], axis=1)
                return jnp.concatenate([top, bot], axis=0).astype(BF16)

            def scores(q, k):
                return jnp.concatenate(
                    [_dot_nt(q[:, 384 * j:384 * (j + 1)], stack(k, j)) for j in range(PP)],
                    axis=0) * scale

            def softmax(sc):
                sc = jnp.where(maskb, sc, _NEG)
                m_lo = jnp.max(jnp.where(lob, sc, -jnp.inf), axis=1, keepdims=True)
                m_hi = jnp.max(jnp.where(lob, -jnp.inf, sc), axis=1, keepdims=True)
                e = jnp.exp(sc - jnp.where(lob, m_lo, m_hi))
                s_lo = jnp.sum(jnp.where(lob, e, 0.0), axis=1, keepdims=True)
                s_hi = jnp.sum(jnp.where(lob, 0.0, e), axis=1, keepdims=True)
                return e / jnp.where(lob, s_lo, s_hi)

            def pv(p, v):
                return jnp.concatenate(
                    [_dot(p[j * L:(j + 1) * L], stack(v, j)) for j in range(PP)], axis=1)

            def out_proj(g, o):
                rows = []
                for j in range(PP):
                    r0 = (g * PP + j) * 2 * Dh
                    rows += [wo_ref[r0:r0 + 128, :], wo_ref[r0 + Dh:r0 + Dh + 128, :],
                             wo_ref[r0 + 128:r0 + Dh, :], wo_ref[r0 + Dh + 128:r0 + 2 * Dh, :]]
                return _dot(o, jnp.concatenate(rows, axis=0))

            qkv = [None] * G
            sc = [None] * G
            p = [None] * G
            o = [None] * G
            acc = None
            for it in range(G + WO_LAG):
                if it < G and not lead:
                    qkv[it] = (proj(0, it), proj(1, it), proj(2, it))
                if 0 <= it - 1 < G:
                    sc[it - 1] = scores(qkv[it - 1][0], qkv[it - 1][1])
                if 0 <= it - 2 < G:
                    o[it - 2] = pv(p[it - 2], qkv[it - 2][2])
                if it < G and lead:
                    qkv[it] = (proj(0, it), proj(1, it), proj(2, it))
                if 0 <= it - 1 < G:
                    p[it - 1] = softmax(sc[it - 1])
                if it == 4:
                    mixer1(x_mix, jnp.where(s >= MD, (s - MD) * SEG, S), SEG)
                if 0 <= it - WO_LAG < G:
                    t = out_proj(it - WO_LAG, o[it - WO_LAG])
                    acc = t if acc is None else acc + t
            xs_ref[r, :] = xs_ref[r, :] + acc[M:, :]
            if layer == 0:
                xs_ref[n_dst, :] = x_next
            ln_ref[n_dst, :] = _ln(x_next)
            return acc[:M, :]

        def lead_steps(i, mem):
            @pl.when(i == XW // UNR)
            def _():
                cp_x1.wait()
            for u in range(UNR):
                mem = a_step(0, True, i * UNR + u, mem)
            return mem

        def b2_in(t):
            r0 = pl.multiple_of(t * RT, RT)
            pieces = []
            shifts = (-1, 1, -2, 2)
            for lt in range(D // 128):
                c0 = lt * 128
                win = h_ref[pl.ds(r0, RT + 2 * HALO), pl.ds(c0, 128)]
                g_lo, g_hi = c0 // c, min((c0 + 127) // c, 3)
                a = win[HALO + shifts[g_lo]: HALO + shifts[g_lo] + RT]
                if g_hi != g_lo:
                    bb = win[HALO + shifts[g_hi]: HALO + shifts[g_hi] + RT]
                    lane = jax.lax.broadcasted_iota(I32, (RT, 128), 1) + c0
                    a = jnp.where(lane < g_hi * c, a, bb)
                pieces.append(a)
            hs_in = jnp.concatenate(pieces, axis=1).astype(BF16)
            return hs_in, xl_ref[pl.ds(r0, RT), :], xs_ref[pl.ds(r0, RT), :]

        def b_tiles(last, i, _):
            ts = [i * BU + u for u in range(BU)]
            ins = [b2_in(t) for t in ts]
            x1 = [xl_t + _dot(hs_in, w2_ref[...]) for hs_in, xl_t, _ in ins]
            for u, t in enumerate(ts):
                g = _gelu(_dot(_ln(x1[u]).astype(BF16), w3_ref[...]))
                xn = ins[u][2] + (x1[u] + _dot(g.astype(BF16), w4_ref[...]))
                r = pl.ds(pl.multiple_of(t * RT, RT), RT)
                if last:
                    x_v[r, :] = xn.astype(BF16)
                else:
                    xs_ref[r, :] = xn
            if last:
                for t in ts:
                    out_copy(t).start()
            return 0

        def out_copy(t):
            r = pl.ds(pl.multiple_of(t * RT, RT), RT)
            return pltpu.make_async_copy(x_v.at[r], out_hbm.at[r], sem_o.at[t])

        for layer in range(2):
            last = layer == 1
            with jax.named_scope('A%d' % layer):
                mem = mem0_ref[...].astype(F32)
                if layer == 0:
                    mem = jax.lax.fori_loop(0, NLEAD // UNR, lead_steps, mem)
                jax.lax.fori_loop(NLEAD if layer == 0 else 0, NSEG,
                                  functools.partial(a_step, layer, False), mem, unroll=UNR)
            if layer == 0:
                for cp in w_cps[2:]:
                    cp.wait()
            with jax.named_scope('B%d' % layer):
                tail = S - MD * SEG
                mixer1(xs_ref[pl.ds(tail, MD * SEG), :], tail, MD * SEG)
                h_ref[pl.ds(HALO + S, HALO), :] = jnp.zeros((HALO, D), F32)
                jax.lax.fori_loop(0, NT // BU, functools.partial(b_tiles, last), 0)
            if not last:
                ln_ref[pl.ds(0, SEG), :] = _ln(xs_ref[pl.ds(0, SEG), :])
        for t in range(NT):
            out_copy(t).wait()

    return kernel


@functools.partial(jax.jit, static_argnames=("A_seg_len",))
def pallas_interleave_layers__memory_aug_recurrent_mem_tr__mixer_s_mlp__prompt_kernel(
    A_x: jax.Array,
    A_mem0: jax.Array,
    A_Wq: jax.Array,
    A_Wk: jax.Array,
    A_Wv: jax.Array,
    A_Wo: jax.Array,
    A_seg_len,
    B_x: jax.Array,
    B_w1: jax.Array,
    B_w2: jax.Array,
    B_w3: jax.Array,
    B_w4: jax.Array,
):
    del B_x
    B, S, D = A_x.shape
    assert B == 1
    H, Dh = A_Wq.shape[1], A_Wq.shape[2]
    M = A_mem0.shape[1]
    SEG = int(A_seg_len)
    F = B_w3.shape[1]
    kernel = _make_kernel(S, D, H, Dh, M, SEG, F)
    hbm = pl.BlockSpec(memory_space=pl.ANY)
    nt = 3 * H // 2

    def wt(w):
        return jnp.transpose(w, (1, 2, 0)).reshape(H * Dh, D)

    out = pl.pallas_call(
        kernel,
        out_shape=jax.ShapeDtypeStruct((S, D), A_x.dtype),
        in_specs=[hbm] * 10,
        out_specs=hbm,
        scratch_shapes=[
            pltpu.VMEM((S, D), BF16),
            pltpu.VMEM((3, H * Dh, D), BF16),
            pltpu.VMEM((nt, D // 2, 128), I32),
            pltpu.VMEM((nt, D // 2, 128), I32),
            pltpu.VMEM((nt, D // 2, 128), I32),
            pltpu.VMEM((H * Dh, D), BF16),
            pltpu.VMEM((D, D), BF16),
            pltpu.VMEM((D, D), BF16),
            pltpu.VMEM((D, F), BF16),
            pltpu.VMEM((F, D), BF16),
            pltpu.VMEM((S + SEG, D), F32),
            pltpu.VMEM((S + SEG, D), F32),
            pltpu.VMEM((S + SEG, D), F32),
            pltpu.VMEM((S + 8 + SEG, D), F32),
            pltpu.VMEM((3, 8, 384, 768), F32),
            pltpu.VMEM((M, D), BF16),
            pltpu.SemaphoreType.DMA((3,)),
            pltpu.SemaphoreType.DMA((48,)),
            pltpu.SemaphoreType.DMA((5,)),
            pltpu.SemaphoreType.DMA((16,)),
        ],
        compiler_params=pltpu.CompilerParams(vmem_limit_bytes=120 * 1024 * 1024),
    )(
        A_mem0.reshape(M, D), A_x.reshape(S, D), wt(A_Wq), wt(A_Wk), wt(A_Wv),
        A_Wo.reshape(H * Dh, D), B_w1, B_w2, B_w3, B_w4,
    )
    return out.reshape(B, S, D)
```

```python
import functools

import jax
import jax.numpy as jnp
import numpy as np
import jax.experimental.pallas as pl
import jax.experimental.pallas.tpu as pltpu

F32 = jnp.float32
BF16 = jnp.bfloat16
I32 = jnp.int32
_NEG = -1000000000.0


def _ln(x, eps=1e-05):
    m = jnp.mean(x, axis=-1, keepdims=True)
    d = x - m
    v = jnp.mean(d * d, axis=-1, keepdims=True)
    return d * jax.lax.rsqrt(v + eps)


def _gelu(x):
    c = float(np.sqrt(2.0 / np.pi))
    return 0.5 * x * (1.0 + jnp.tanh(c * (x + 0.044715 * (x * x * x))))


def _dot(a, b):
    return jnp.dot(a, b, preferred_element_type=F32)


def _dot_nt(a, b):
    return jax.lax.dot_general(a, b, (((1,), (1,)), ((), ())), preferred_element_type=F32)


def _make_kernel(S, D, H, Dh, M, SEG, G=8, WO_LAG=4, RAMP=4, UNR=2, BU=2, MD=2):
    L = M + SEG
    NSEG = S // SEG
    NP = H // 2
    PP = NP // G
    scale = Dh ** (-0.5)
    RT = 128
    NT = S // RT
    HALO = 8
    c = D // 4
    PW = 2 * Dh
    AHEAD = RAMP + 1
    XR = 24
    LEAD = 12 * XR
    NLEAD = LEAD // (SEG - XR)
    RING = 384
    X0 = LEAD + XR
    XW = 8
    X1 = X0 + XW * XR + 8
    assert (S, D, H, Dh, M, SEG) == (2048, 640, 32, 192, 8, 32)
    assert NLEAD % UNR == 0 and XW % UNR == 0
    assert RING % XR == 0 and RING % SEG == 0 and RING >= LEAD + XR

    def kernel(mem0_hbm, x_hbm, wq_hbm, wk_hbm, wv_hbm, wo_hbm,
               w1_hbm, w2_hbm, w3_hbm, w4_hbm, out_hbm,
               x_v, stage, wq_s, wk_s, wv_s, wo_ref, w1_ref, w2_ref, w3_ref, w4_ref,
               xs_ref, ln_ref, xl_ref, h_ref, ring, mem0_ref, sem_x, sem_st, sem_w, sem_o):
        def st_copy(j, mi):
            rows = pl.ds(pl.multiple_of(j * PW, 128), PW)
            return pltpu.make_async_copy(
                (wq_hbm, wk_hbm, wv_hbm)[mi].at[rows], stage.at[mi, rows], sem_st.at[3 * j + mi])

        cp_x0 = pltpu.make_async_copy(x_hbm.at[pl.ds(0, X1)], x_v.at[pl.ds(0, X1)], sem_x.at[0])
        cp_x1 = pltpu.make_async_copy(
            x_hbm.at[pl.ds(X1, S - X1)], x_v.at[pl.ds(X1, S - X1)], sem_x.at[1])
        w_cps = [pltpu.make_async_copy(src, dst, sem_w.at[wi])
                 for wi, (src, dst) in enumerate(
                     ((wo_hbm, wo_ref), (w1_hbm, w1_ref), (w2_hbm, w2_ref),
                      (w3_hbm, w3_ref), (w4_hbm, w4_ref)))]
        cp_x0.start()
        for j in range(2):
            for mi in range(3):
                st_copy(j, mi).start()
        cp_m = pltpu.make_async_copy(mem0_hbm, mem0_ref, sem_x.at[2])
        cp_m.start()

        def prenorm(r):
            x = x_v[r, :].astype(F32)
            xs_ref[r, :] = x
            ln_ref[r, :] = _ln(x)

        cp_x0.wait()
        prenorm(pl.ds(0, X0))
        h_ref[pl.ds(0, HALO), :] = jnp.zeros((HALO, D), F32)

        def relayout(j):
            r0 = pl.multiple_of(j * PW, 128)
            for mi, dst in enumerate((wq_s, wk_s, wv_s)):
                a = stage[mi, pl.ds(r0, 128), :]
                b = stage[mi, pl.ds(r0 + Dh, 128), :]
                t = jnp.concatenate([stage[mi, pl.ds(r0 + 128, 64), :],
                                     stage[mi, pl.ds(r0 + Dh + 128, 64), :]], axis=0)
                for n, v in enumerate((a, b, t)):
                    dst[3 * j + n] = pltpu.bitcast(v.T, I32)

        def pair_w(w_s, j):
            return jnp.concatenate(
                [pltpu.bitcast(w_s[3 * j + t], BF16) for t in range(3)], axis=1)

        def lead_proj(j):
            rows = ln_ref[pl.ds(0, LEAD), :]
            for mi, w_s in enumerate((wq_s, wk_s, wv_s)):
                cols = pl.ds(pl.multiple_of((j % PP) * PW, 128), PW)
                ring[mi, j // PP, pl.ds(0, LEAD), cols] = _dot(rows, pair_w(w_s, j))

        def arrive(j):
            for mi in range(3):
                st_copy(j, mi).wait()

            @pl.when(j + AHEAD < NP)
            def _():
                for mi in range(3):
                    st_copy(j + AHEAD, mi).start()

            @pl.when(j + AHEAD == NP)
            def _():
                w_cps[0].start()
                w_cps[1].start()

        for j in range(2, RAMP + 1):
            for mi in range(3):
                st_copy(j - 2, mi).wait()
                st_copy(2 * j - 2, mi).start()
                st_copy(2 * j - 1, mi).start()
            relayout(j - 2)
            if j > 2:
                lead_proj(j - 3)

        def startup(j, _):
            arrive(j)
            lead_proj(j - 1)
            relayout(j)
            return 0
        jax.lax.fori_loop(RAMP - 1, NP, startup, 0)
        lead_proj(NP - 1)
        cp_m.wait()
        w_cps[0].wait()
        w_cps[1].wait()
        cp_x1.start()
        for cp in w_cps[2:]:
            cp.start()

        def mixer1(x, dst, n):
            xl = _ln(x)
            xl_ref[pl.ds(pl.multiple_of(dst, 8), n), :] = xl
            h_ref[pl.ds(pl.multiple_of(dst + HALO, 8), n), :] = _gelu(
                _dot(_ln(xl).astype(BF16), w1_ref[...]))

        def a_step(layer, lead, s, mem):
            r = pl.ds(pl.multiple_of(s * SEG, SEG), SEG)
            m_src = pl.ds(pl.multiple_of(jnp.maximum(s - MD, 0) * SEG, SEG), SEG)
            x_mix = xs_ref[m_src, :]
            n0 = X0 + s * XR if lead else (s + 1) * SEG
            n_src = pl.ds(pl.multiple_of(jnp.minimum(n0, S - SEG), 8), SEG)
            n_dst = pl.ds(pl.multiple_of(n0, 8), SEG)
            if layer == 0:
                x_next = x_v[n_src, :].astype(F32)
            else:
                x_next = xs_ref[n_src, :]
            if lead:
                p0 = LEAD + s * XR
                hrows = jnp.concatenate(
                    [mem, ln_ref[pl.ds(pl.multiple_of(p0, 8), XR), :]], axis=0).astype(BF16)
                wpos = pl.ds(pl.multiple_of(jax.lax.rem(p0, RING), 8), XR)
                rpos = pl.ds(pl.multiple_of(jax.lax.rem(s * SEG, RING), 8), SEG)
            else:
                hrows = jnp.concatenate([mem, ln_ref[r, :]], axis=0)
            lo64 = jax.lax.broadcasted_iota(I32, (L, 128), 1) < 64
            zero = jnp.zeros((L, 128), F32)
            rowb = jax.lax.broadcasted_iota(I32, (PP * L, 2 * L), 0) % L
            colb = jax.lax.broadcasted_iota(I32, (PP * L, 2 * L), 1)
            lob = colb < L
            maskb = (rowb < M) | (rowb >= jnp.where(lob, colb, colb - L))

            def proj(mi, g):
                w_s = (wq_s, wk_s, wv_s)[mi]
                y = _dot(hrows, jnp.concatenate(
                    [pair_w(w_s, g * PP + u) for u in range(PP)], axis=1))
                if lead:
                    ring[mi, g, wpos, :] = y[M:, :]
                    y = jnp.concatenate([y[:M, :], ring[mi, g, rpos, :]], axis=0)
                return y

            def stack(x, j):
                t0 = x[:, 384 * j:384 * j + 128]
                t1 = x[:, 384 * j + 128:384 * j + 256]
                t2 = x[:, 384 * j + 256:384 * j + 384]
                top = jnp.concatenate([t0, zero, jnp.where(lo64, t2, 0.0)], axis=1)
                bot = jnp.concatenate([zero, t1, jnp.where(lo64, 0.0, t2)], axis=1)
                return jnp.concatenate([top, bot], axis=0).astype(BF16)

            def scores(q, k):
                return jnp.concatenate(
                    [_dot_nt(q[:, 384 * j:384 * (j + 1)], stack(k, j)) for j in range(PP)],
                    axis=0) * scale

            def softmax(sc):
                sc = jnp.where(maskb, sc, _NEG)
                m_lo = jnp.max(jnp.where(lob, sc, -jnp.inf), axis=1, keepdims=True)
                m_hi = jnp.max(jnp.where(lob, -jnp.inf, sc), axis=1, keepdims=True)
                e = jnp.exp(sc - jnp.where(lob, m_lo, m_hi))
                s_lo = jnp.sum(jnp.where(lob, e, 0.0), axis=1, keepdims=True)
                s_hi = jnp.sum(jnp.where(lob, 0.0, e), axis=1, keepdims=True)
                return e / jnp.where(lob, s_lo, s_hi)

            def pv(p, v):
                return jnp.concatenate(
                    [_dot(p[j * L:(j + 1) * L], stack(v, j)) for j in range(PP)], axis=1)

            def out_proj(g, o):
                rows = []
                for j in range(PP):
                    r0 = (g * PP + j) * 2 * Dh
                    rows += [wo_ref[r0:r0 + 128, :], wo_ref[r0 + Dh:r0 + Dh + 128, :],
                             wo_ref[r0 + 128:r0 + Dh, :], wo_ref[r0 + Dh + 128:r0 + 2 * Dh, :]]
                return _dot(o, jnp.concatenate(rows, axis=0))

            qkv = [None] * G
            sc = [None] * G
            p = [None] * G
            o = [None] * G
            acc = None
            for it in range(G + WO_LAG):
                if it < G and not lead:
                    qkv[it] = (proj(0, it), proj(1, it), proj(2, it))
                if 0 <= it - 1 < G:
                    sc[it - 1] = scores(qkv[it - 1][0], qkv[it - 1][1])
                if 0 <= it - 2 < G:
                    o[it - 2] = pv(p[it - 2], qkv[it - 2][2])
                if it < G and lead:
                    qkv[it] = (proj(0, it), proj(1, it), proj(2, it))
                if 0 <= it - 1 < G:
                    p[it - 1] = softmax(sc[it - 1])
                if it == 4:
                    mixer1(x_mix, jnp.where(s >= MD, (s - MD) * SEG, S), SEG)
                if 0 <= it - WO_LAG < G:
                    t = out_proj(it - WO_LAG, o[it - WO_LAG])
                    acc = t if acc is None else acc + t
            xs_ref[r, :] = xs_ref[r, :] + acc[M:, :]
            if layer == 0:
                xs_ref[n_dst, :] = x_next
            ln_ref[n_dst, :] = _ln(x_next)
            return acc[:M, :]

        def lead_steps(i, mem):
            @pl.when(i == XW // UNR)
            def _():
                cp_x1.wait()
            for u in range(UNR):
                mem = a_step(0, True, i * UNR + u, mem)
            return mem

        def b2_in(t):
            r0 = pl.multiple_of(t * RT, RT)
            pieces = []
            shifts = (-1, 1, -2, 2)
            for lt in range(D // 128):
                c0 = lt * 128
                win = h_ref[pl.ds(r0, RT + 2 * HALO), pl.ds(c0, 128)]
                g_lo, g_hi = c0 // c, min((c0 + 127) // c, 3)
                a = win[HALO + shifts[g_lo]: HALO + shifts[g_lo] + RT]
                if g_hi != g_lo:
                    bb = win[HALO + shifts[g_hi]: HALO + shifts[g_hi] + RT]
                    lane = jax.lax.broadcasted_iota(I32, (RT, 128), 1) + c0
                    a = jnp.where(lane < g_hi * c, a, bb)
                pieces.append(a)
            hs_in = jnp.concatenate(pieces, axis=1).astype(BF16)
            return hs_in, xl_ref[pl.ds(r0, RT), :], xs_ref[pl.ds(r0, RT), :]

        def b_tiles(last, i, _):
            ts = [i * BU + u for u in range(BU)]
            ins = [b2_in(t) for t in ts]
            x1 = [xl_t + _dot(hs_in, w2_ref[...]) for hs_in, xl_t, _ in ins]
            for u, t in enumerate(ts):
                g = _gelu(_dot(_ln(x1[u]).astype(BF16), w3_ref[...]))
                xn = ins[u][2] + (x1[u] + _dot(g.astype(BF16), w4_ref[...]))
                r = pl.ds(pl.multiple_of(t * RT, RT), RT)
                if last:
                    x_v[r, :] = xn.astype(BF16)
                else:
                    xs_ref[r, :] = xn
            if last:
                for t in ts:
                    out_copy(t).start()
            return 0

        def out_copy(t):
            r = pl.ds(pl.multiple_of(t * RT, RT), RT)
            return pltpu.make_async_copy(x_v.at[r], out_hbm.at[r], sem_o.at[t])

        for layer in range(2):
            last = layer == 1
            mem = mem0_ref[...].astype(F32)
            if layer == 0:
                mem = jax.lax.fori_loop(0, NLEAD // UNR, lead_steps, mem)
            jax.lax.fori_loop(NLEAD if layer == 0 else 0, NSEG,
                              functools.partial(a_step, layer, False), mem, unroll=UNR)
            if layer == 0:
                for cp in w_cps[2:]:
                    cp.wait()
            tail = S - MD * SEG
            mixer1(xs_ref[pl.ds(tail, MD * SEG), :], tail, MD * SEG)
            h_ref[pl.ds(HALO + S, HALO), :] = jnp.zeros((HALO, D), F32)
            jax.lax.fori_loop(0, NT // BU, functools.partial(b_tiles, last), 0)
            if not last:
                ln_ref[pl.ds(0, SEG), :] = _ln(xs_ref[pl.ds(0, SEG), :])
        for t in range(NT):
            out_copy(t).wait()

    return kernel


@functools.partial(jax.jit, static_argnames=("A_seg_len",))
def pallas_interleave_layers__memory_aug_recurrent_mem_tr__mixer_s_mlp__prompt_kernel(
    A_x: jax.Array,
    A_mem0: jax.Array,
    A_Wq: jax.Array,
    A_Wk: jax.Array,
    A_Wv: jax.Array,
    A_Wo: jax.Array,
    A_seg_len,
    B_x: jax.Array,
    B_w1: jax.Array,
    B_w2: jax.Array,
    B_w3: jax.Array,
    B_w4: jax.Array,
):
    del B_x
    B, S, D = A_x.shape
    assert B == 1
    H, Dh = A_Wq.shape[1], A_Wq.shape[2]
    M = A_mem0.shape[1]
    SEG = int(A_seg_len)
    F = B_w3.shape[1]
    kernel = _make_kernel(S, D, H, Dh, M, SEG)
    hbm = pl.BlockSpec(memory_space=pl.ANY)
    nt = 3 * H // 2

    def wt(w):
        return jnp.transpose(w, (1, 2, 0)).reshape(H * Dh, D)

    out = pl.pallas_call(
        kernel,
        out_shape=jax.ShapeDtypeStruct((S, D), A_x.dtype),
        in_specs=[hbm] * 10,
        out_specs=hbm,
        scratch_shapes=[
            pltpu.VMEM((S, D), BF16),
            pltpu.VMEM((3, H * Dh, D), BF16),
            pltpu.VMEM((nt, D // 2, 128), I32),
            pltpu.VMEM((nt, D // 2, 128), I32),
            pltpu.VMEM((nt, D // 2, 128), I32),
            pltpu.VMEM((H * Dh, D), BF16),
            pltpu.VMEM((D, D), BF16),
            pltpu.VMEM((D, D), BF16),
            pltpu.VMEM((D, F), BF16),
            pltpu.VMEM((F, D), BF16),
            pltpu.VMEM((S + SEG, D), F32),
            pltpu.VMEM((S + SEG, D), F32),
            pltpu.VMEM((S + SEG, D), F32),
            pltpu.VMEM((S + 8 + SEG, D), F32),
            pltpu.VMEM((3, 8, 384, 768), F32),
            pltpu.VMEM((M, D), BF16),
            pltpu.SemaphoreType.DMA((3,)),
            pltpu.SemaphoreType.DMA((48,)),
            pltpu.SemaphoreType.DMA((5,)),
            pltpu.SemaphoreType.DMA((16,)),
        ],
        compiler_params=pltpu.CompilerParams(vmem_limit_bytes=120 * 1024 * 1024),
    )(
        A_mem0.reshape(M, D), A_x.reshape(S, D), wt(A_Wq), wt(A_Wk), wt(A_Wv),
        A_Wo.reshape(H * Dh, D), B_w1, B_w2, B_w3, B_w4,
    )
    return out.reshape(B, S, D)
```
